```python
import jax
import jax.numpy as jnp

def _softmax(x, axis=-1):
    return jax.nn.softmax(x, axis=axis)

def _gelu(x):
    return jax.nn.gelu(x, approximate=True)

def _silu(x):
    return jax.nn.silu(x)

def _sigmoid(x):
    return jax.nn.sigmoid(x)

def _layernorm(x, axis=-1, eps=1e-05):
    m = jnp.mean(x, axis=axis, keepdims=True)
    v = jnp.var(x, axis=axis, keepdims=True)
    return (x - m) / jnp.sqrt(v + eps)

def _scatter_add(tgt, idx, src, axis=0):
    return tgt.at[idx].add(src)

def _segment_sum(src, seg, n):
    return jax.ops.segment_sum(src, seg, n)

class _Rng:

    def __init__(self, key):
        self._k = key

    def _next(self):
        self._k, sub = jax.random.split(self._k)
        return sub

    def normal(self, shape):
        return jax.random.normal(self._next(), shape, dtype=jnp.bfloat16)

    def randint(self, lo, hi, shape):
        return jax.random.randint(self._next(), shape, lo, hi, dtype=jnp.int32)

    def uniform(self, shape, lo=0.0, hi=1.0):
        return jax.random.uniform(self._next(), shape, jnp.bfloat16, lo, hi)

    def permutation(self, n):
        return jax.random.permutation(self._next(), n)
kernel_name = 'interleave_layers__memory_aug_recurrent_mem_tr__glu_gated_swiglu__prompt'

def setup_inputs():
    _rng = _Rng(jax.random.key(int.from_bytes(__import__("os").urandom(4), "little")))
    _w = lambda a: (lambda t: t.astype(jnp.bfloat16) if jnp.issubdtype(t.dtype, jnp.floating) else t)(jnp.asarray(a))

    def _A_setup():
        B, S, Dm = (1, 2048, 576)
        H, Dh = (32, 128)
        M, seg = (8, 32)
        seg = min(seg, S)
        S = S // seg * seg
        return {'x': _w((lambda *s: _rng.normal(s) * 0.05)(B, S, Dm)), 'mem0': _w((lambda *s: _rng.normal(s) * 0.05)(B, M, Dm)), 'Wq': _w((lambda *s: _rng.normal(s) * 0.05)(Dm, H, Dh) * Dm ** (-0.5)), 'Wk': _w((lambda *s: _rng.normal(s) * 0.05)(Dm, H, Dh) * Dm ** (-0.5)), 'Wv': _w((lambda *s: _rng.normal(s) * 0.05)(Dm, H, Dh) * Dm ** (-0.5)), 'Wo': _w((lambda *s: _rng.normal(s) * 0.05)(H, Dh, Dm) * (H * Dh) ** (-0.5)), 'seg_len': seg}
    _A_in = _A_setup()

    def _B_setup():
        B, S, D, F = (1, 2048, 576, 4608)
        return {'x': _w((lambda *s: _rng.normal(s) * 0.05)(B, S, D)), 'w1': _w((lambda *s: _rng.normal(s) * 0.05)(D, F) * (2.0 / D) ** 0.5), 'w3': _w((lambda *s: _rng.normal(s) * 0.05)(D, F) * (2.0 / D) ** 0.5), 'w2': _w((lambda *s: _rng.normal(s) * 0.05)(F, D) * (2.0 / F) ** 0.5)}
    _B_in = _B_setup()
    return {'A_x': _A_in['x'], 'A_mem0': _A_in['mem0'], 'A_Wq': _A_in['Wq'], 'A_Wk': _A_in['Wk'], 'A_Wv': _A_in['Wv'], 'A_Wo': _A_in['Wo'], 'A_seg_len': _A_in['seg_len'], 'B_x': _B_in['x'], 'B_w1': _B_in['w1'], 'B_w3': _B_in['w3'], 'B_w2': _B_in['w2']}

def reference(A_x, A_mem0, A_Wq, A_Wk, A_Wv, A_Wo, A_seg_len, B_x, B_w1, B_w3, B_w2):

    def _A_ref(x, mem0, Wq, Wk, Wv, Wo, seg_len):
        B, S, Dm = x.shape
        H, Dh = (Wq.shape[1], Wq.shape[2])
        M = mem0.shape[1]
        scale = Dh ** (-0.5)
        n_seg = S // seg_len
        L = M + seg_len
        idx = jnp.arange(L)
        mask = (idx[:, None] < M) | (idx[:, None] >= idx[None, :])
        mem = mem0
        outs = []
        for s in range(n_seg):
            xs = x[:, s * seg_len:(s + 1) * seg_len, :].copy()
            h = jnp.concatenate([mem, xs], axis=1)
            q = jnp.einsum('btd,dhe->bhte', h, Wq)
            k = jnp.einsum('btd,dhe->bhte', h, Wk)
            v = jnp.einsum('btd,dhe->bhte', h, Wv)
            scores = jnp.einsum('bhqe,bhke->bhqk', q, k) * scale
            scores = jnp.where(mask[None, None], scores, -1000000000.0)
            p = _softmax(scores, axis=-1)
            o = jnp.einsum('bhqk,bhke->bhqe', p, v)
            o = jnp.einsum('bhte,hed->btd', o, Wo)
            mem = o[:, :M, :].copy()
            outs.append(o[:, M:, :])
        return jnp.concatenate(outs, axis=1)

    def _B_ref(x, w1, w3, w2):
        gate = jnp.einsum('bsd,df->bsf', x, w1)
        up = jnp.einsum('bsd,df->bsf', x, w3)
        h = _silu(gate) * up
        out = jnp.einsum('bsf,fd->bsd', h, w2)
        return out
    x = A_x
    x = x + _A_ref(_layernorm(x, axis=-1), A_mem0, A_Wq, A_Wk, A_Wv, A_Wo, A_seg_len)
    x = x + _B_ref(_layernorm(x, axis=-1), B_w1, B_w3, B_w2)
    x = x + _A_ref(_layernorm(x, axis=-1), A_mem0, A_Wq, A_Wk, A_Wv, A_Wo, A_seg_len)
    x = x + _B_ref(_layernorm(x, axis=-1), B_w1, B_w3, B_w2)
    return x
```

```python
import functools
import math

import jax
import jax.numpy as jnp
import jax.experimental.pallas as pl
import jax.experimental.pallas.tpu as pltpu
import numpy as np

_EPS = 1e-05
_MASKED = -1000000000.0
_LOG2E = math.log2(math.e)
_HEADS_PER_GROUP = 4
_FFN_CHUNK = 512


def _layernorm(x):
    m = jnp.mean(x, axis=-1, keepdims=True)
    d = x - m
    v = jnp.mean(d * d, axis=-1, keepdims=True)
    return d * jax.lax.rsqrt(v + _EPS)


def _dot(a, b):
    return jnp.dot(a, b, preferred_element_type=jnp.float32)


def _attention_masks(n_mem, seg):
    rows = 2 * (n_mem + seg)
    i = jax.lax.broadcasted_iota(jnp.int32, (rows, rows), 0)
    j = jax.lax.broadcasted_iota(jnp.int32, (rows, rows), 1)

    def second_layer(r):
        return ((r >= n_mem) & (r < 2 * n_mem)) | (r >= 2 * n_mem + seg)

    same = second_layer(i) == second_layer(j)
    visible = same & ((i < 2 * n_mem) | (i >= j))
    fill = jnp.where(same, _MASKED * _LOG2E, -jnp.inf).astype(jnp.float32)
    return visible, fill


def _kernel(x_hbm, mem0_ref, wq_hbm, wk_hbm, wv_hbm, wo_hbm, w1_hbm, w3_hbm, w2_hbm,
            out_hbm, x_ref, out_ref, stage_ref, wqkv_ref, wo_ref, w1_ref, w3_ref, w2_ref,
            stage_sem, sem, *, seg):
    n_tok, d_model = x_ref.shape
    n_mem = mem0_ref.shape[0]
    n_pairs, _, d_head = stage_ref.shape[1:]
    n_heads = 2 * n_pairs
    d_ff = w1_ref.shape[1]
    n_seg = n_tok // seg
    scale = d_head ** -0.5

    head_copies = [
        [pltpu.make_async_copy(w.bitcast(jnp.uint32).at[:, p, :], stage_ref.at[i, p],
                               stage_sem.at[i * n_pairs + p])
         for i, w in enumerate((wq_hbm, wk_hbm, wv_hbm))]
        for p in range(n_pairs)]
    copies = [pltpu.make_async_copy(src, dst, sem.at[i]) for i, (src, dst) in enumerate((
        (x_hbm, x_ref), (wo_hbm, wo_ref), (w1_hbm, w1_ref), (w3_hbm, w3_ref), (w2_hbm, w2_ref)))]
    copies[0].start()
    for group in head_copies:
        for c in group:
            c.start()
    for c in copies[1:]:
        c.start()
    for p in range(n_pairs):
        for i in range(3):
            head_copies[p][i].wait()
            words = stage_ref[i, p]
            lo = pltpu.bitcast(words << 16, jnp.float32)
            hi = pltpu.bitcast(words & jnp.uint32(0xFFFF0000), jnp.float32)
            for half, w in enumerate((lo, hi)):
                col = (3 * (2 * p + half) + i) * d_head
                wqkv_ref[:, col:col + d_head] = w.astype(jnp.bfloat16)
    for c in copies:
        c.wait()

    visible, fill = _attention_masks(n_mem, seg)
    mem0 = mem0_ref[...].astype(jnp.float32)
    group_cols = 3 * d_head * _HEADS_PER_GROUP

    def attend(qkv):
        outs = []
        for h in range(_HEADS_PER_GROUP):
            q, k, v = (qkv[:, (3 * h + i) * d_head:(3 * h + i + 1) * d_head] for i in range(3))
            s = jax.lax.dot_general(q, k, (((1,), (1,)), ((), ())),
                                    preferred_element_type=jnp.float32)
            s = jnp.where(visible, s * (scale * _LOG2E), fill)
            p = jnp.exp2(s - jnp.max(s, axis=-1, keepdims=True))
            inv = 1.0 / jnp.sum(p, axis=-1, keepdims=True)
            outs.append((_dot(p.astype(jnp.bfloat16), v) * inv).astype(jnp.bfloat16))
        return outs

    def step(t, carry):
        mem, x2 = carry
        row1 = pl.multiple_of(jnp.minimum(t, n_seg - 1) * seg, seg)
        x1 = x_ref[pl.ds(row1, seg), :].astype(jnp.float32)
        xin = jnp.concatenate([x1, x2], axis=0)
        h = jnp.concatenate([mem, _layernorm(xin)], axis=0).astype(jnp.bfloat16)

        heads = []
        n_groups = n_heads // _HEADS_PER_GROUP
        project = lambda g: _dot(
            h, wqkv_ref[:, g * group_cols:(g + 1) * group_cols]).astype(jnp.bfloat16)
        qkv = project(0)
        for g in range(n_groups):
            nxt = project(g + 1) if g + 1 < n_groups else None
            heads += attend(qkv)
            qkv = nxt
        out = _dot(jnp.concatenate(heads, axis=1), wo_ref[...])

        mem_next = jnp.concatenate(
            [out[:n_mem], jnp.where(t == 0, mem0, out[n_mem:2 * n_mem])], axis=0)
        xa = xin + out[2 * n_mem:]
        hn = _layernorm(xa).astype(jnp.bfloat16)
        acts = []
        for c in range(0, d_ff, _FFN_CHUNK):
            gate = _dot(hn, w1_ref[:, c:c + _FFN_CHUNK])
            up = _dot(hn, w3_ref[:, c:c + _FFN_CHUNK])
            acts.append((gate * jax.nn.sigmoid(gate) * up).astype(jnp.bfloat16))
        xb = xa + _dot(jnp.concatenate(acts, axis=1), w2_ref[...])

        row2 = pl.multiple_of(jnp.maximum(t - 1, 0) * seg, seg)
        out_ref[pl.ds(row2, seg), :] = xb[seg:].astype(out_ref.dtype)
        return mem_next, xb[:seg]

    init = (jnp.concatenate([mem0, mem0], axis=0), jnp.zeros((seg, d_model), jnp.float32))
    jax.lax.fori_loop(0, n_seg + 1, step, init)

    store = pltpu.make_async_copy(out_ref, out_hbm, sem.at[0])
    store.start()
    store.wait()


@functools.partial(jax.jit, static_argnames=("A_seg_len",))
def pallas_interleave_layers__memory_aug_recurrent_mem_tr__glu_gated_swiglu__prompt_kernel(
    A_x: jax.Array,
    A_mem0: jax.Array,
    A_Wq: jax.Array,
    A_Wk: jax.Array,
    A_Wv: jax.Array,
    A_Wo: jax.Array,
    A_seg_len: int,
    B_x: jax.Array,
    B_w1: jax.Array,
    B_w3: jax.Array,
    B_w2: jax.Array,
):
    del B_x
    _, n_tok, d_model = A_x.shape
    n_mem = A_mem0.shape[1]
    _, n_heads, d_head = A_Wq.shape
    d_ff = B_w1.shape[1]
    bf16 = jnp.bfloat16
    hbm = pl.BlockSpec(memory_space=pl.ANY)
    out = pl.pallas_call(
        functools.partial(_kernel, seg=A_seg_len),
        out_shape=jax.ShapeDtypeStruct((n_tok, d_model), A_x.dtype),
        in_specs=[hbm, pl.BlockSpec(memory_space=pltpu.VMEM)] + [hbm] * 7,
        out_specs=hbm,
        scratch_shapes=[
            pltpu.VMEM((n_tok, d_model), A_x.dtype),
            pltpu.VMEM((n_tok, d_model), A_x.dtype),
            pltpu.VMEM((3, n_heads // 2, d_model, d_head), jnp.uint32),
            pltpu.VMEM((d_model, 3 * n_heads * d_head), bf16),
            pltpu.VMEM((n_heads * d_head, d_model), bf16),
            pltpu.VMEM((d_model, d_ff), bf16),
            pltpu.VMEM((d_model, d_ff), bf16),
            pltpu.VMEM((d_ff, d_model), bf16),
            pltpu.SemaphoreType.DMA((3 * n_heads // 2,)),
            pltpu.SemaphoreType.DMA((5,)),
        ],
        compiler_params=pltpu.CompilerParams(vmem_limit_bytes=100 * 1024 * 1024),
    )(A_x.reshape(n_tok, d_model), A_mem0.reshape(n_mem, d_model), A_Wq, A_Wk, A_Wv,
      A_Wo.reshape(n_heads * d_head, d_model), B_w1, B_w3, B_w2)
    return out.reshape(A_x.shape)
```

```python
import functools
import math

import jax
import jax.numpy as jnp
import jax.experimental.pallas as pl
import jax.experimental.pallas.tpu as pltpu

_EPS = 1e-05
_MASKED = -1000000000.0
_LOG2E = math.log2(math.e)
_LANES = 128
_LAG = 4
_EARLY = 8
_HEADS_PER_GROUP = 4
_FFN_CHUNK = 512
_COPIES_AHEAD = 4
_FFN_COPY_LEAD = 1
_PIPELINE = (("P", 2), ("S", 1), ("X", 1), ("V", 0), ("G", 0), ("O", -1))
_MAX_SKEW = 4


def _layernorm(x):
    m = jnp.mean(x, axis=-1, keepdims=True)
    d = x - m
    v = jnp.mean(d * d, axis=-1, keepdims=True)
    return d * jax.lax.rsqrt(v + _EPS)


def _dot(a, b):
    return jnp.dot(a, b, preferred_element_type=jnp.float32)


def _dot_nt(a, b):
    return jax.lax.dot_general(a, b, (((1,), (1,)), ((), ())),
                               preferred_element_type=jnp.float32)


def _pack(x):
    return pltpu.bitcast(x, jnp.uint32)


def _unpack(words):
    return pltpu.bitcast(words, jnp.bfloat16)


def _attention_masks(n_layers, n_mem, seg):
    rows = n_layers * (n_mem + seg)
    i = jax.lax.broadcasted_iota(jnp.int32, (rows, rows), 0)
    j = jax.lax.broadcasted_iota(jnp.int32, (rows, rows), 1)
    visible = (i < n_layers * n_mem) | (i >= j)
    if n_layers == 1:
        return visible, _MASKED * _LOG2E

    def second_layer(r):
        return ((r >= n_mem) & (r < 2 * n_mem)) | (r >= 2 * n_mem + seg)

    same = second_layer(i) == second_layer(j)
    fill = jnp.where(same, _MASKED * _LOG2E, -jnp.inf).astype(jnp.float32)
    return same & visible, fill


def _kernel(xt_hbm, mem0_ref, wq_hbm, wk_hbm, wv_hbm, wot_hbm, w1_hbm, w3_hbm, w2t_hbm,
            outt_hbm, xt_ref, res_ref, h_ref, early_ref, stage_ref, wqkv_ref, wot_ref, w1_ref,
            w3_ref, w2t_ref, stage_sem, wo_sem, out_sem, sem, *, seg):
    d_model, n_tok = xt_ref.shape
    n_mem = mem0_ref.shape[0]
    n_pairs, _, d_head = stage_ref.shape[1:]
    n_heads = 2 * n_pairs
    n_groups = n_heads // _HEADS_PER_GROUP
    group_cols = 3 * d_head * _HEADS_PER_GROUP
    n_chunks = w1_ref.shape[1] // _FFN_CHUNK
    n_seg = n_tok // seg
    n_io = n_tok // _LANES
    score_scale = d_head ** -0.5 * _LOG2E

    def block(r):
        return pl.ds(pl.multiple_of(r * seg, seg), seg)

    def load_blocks(blocks):
        return jnp.concatenate([res_ref[block(r), :] for r in blocks], axis=0)

    def store_blocks(blocks, value):
        for i, r in enumerate(blocks):
            res_ref[block(r), :] = value[i * seg:(i + 1) * seg]

    def normed(blocks):
        return _layernorm(load_blocks(blocks)).astype(jnp.bfloat16)

    def mix(project, attn_blocks, ffn_blocks):
        n_layers = len(attn_blocks)
        if attn_blocks:
            visible, fill = _attention_masks(n_layers, n_mem, seg)
        if ffn_blocks:
            y = load_blocks(ffn_blocks)
            hn = _layernorm(y).astype(jnp.bfloat16)
        qkv, scores, probs, heads, acts, out = {}, {}, {}, {}, [], None

        def part(g, head, which):
            col = (3 * head + which) * d_head
            return qkv[g][:, col:col + d_head]

        for it in range(-_MAX_SKEW, max(n_groups, n_chunks) + _MAX_SKEW):
            for stage, skew in _PIPELINE:
                g = it + skew
                if stage == "G":
                    if ffn_blocks and 0 <= g < n_chunks:
                        cols = slice(g * _FFN_CHUNK, (g + 1) * _FFN_CHUNK)
                        gate = _dot(hn, _unpack(w1_ref[:, cols]))
                        up = _dot(hn, _unpack(w3_ref[:, cols]))
                        acts.append((gate * jax.nn.sigmoid(gate) * up).astype(jnp.bfloat16))
                elif not (attn_blocks and 0 <= g < n_groups):
                    continue
                elif stage == "P":
                    qkv[g] = project(slice(g * group_cols, (g + 1) * group_cols))
                elif stage == "S":
                    scores[g] = [_dot_nt(part(g, i, 0), part(g, i, 1))
                                 for i in range(_HEADS_PER_GROUP)]
                elif stage == "X":
                    probs[g] = []
                    for s in scores[g]:
                        s = jnp.where(visible, s * score_scale, fill)
                        p = jnp.exp2(s - jnp.max(s, axis=-1, keepdims=True))
                        inv = 1.0 / jnp.sum(p, axis=-1, keepdims=True)
                        probs[g].append((p.astype(jnp.bfloat16), inv))
                elif stage == "V":
                    heads[g] = [(_dot(p, part(g, i, 2)) * inv).astype(jnp.bfloat16)
                                for i, (p, inv) in enumerate(probs[g])]
                elif stage == "O":
                    width = _HEADS_PER_GROUP * d_head
                    o = _dot_nt(jnp.concatenate(heads[g], axis=1),
                                _unpack(wot_ref[:, g * width:(g + 1) * width]))
                    out = o if out is None else out + o
        mems = xa = None
        if ffn_blocks:
            y = y + _dot_nt(jnp.concatenate(acts, axis=1), _unpack(w2t_ref[...]))
        if attn_blocks:
            mems = out[:n_layers * n_mem]
            xa = load_blocks(attn_blocks) + out[n_layers * n_mem:]
            store_blocks(attn_blocks, xa)
        if ffn_blocks:
            store_blocks([r + n_seg for r in ffn_blocks], y)
        return mems

    def projector(h):
        return lambda cols: _dot(h, _unpack(wqkv_ref[:, cols])).astype(jnp.bfloat16)

    def single_step(r, mem, ffn_blocks=()):
        h = jnp.concatenate([mem, _layernorm(load_blocks([r]))], axis=0)
        return mix(projector(h.astype(jnp.bfloat16)), [r], ffn_blocks)

    def ffn_step(blocks):
        mix(None, [], blocks)

    def double_step(b, _, *, early):
        ffn_blocks = [jnp.where(b == 0, _LAG - 2, b + _LAG - 1),
                      jnp.where(b == 0, _LAG - 1, n_seg + b - 1)]
        h_next = normed([jnp.minimum(b + 1 + _LAG, n_seg - 1), n_seg + b + 1])
        if early:
            rest = projector(jnp.concatenate(
                [h_ref[:2 * n_mem, :], h_ref[2 * n_mem + seg:, :]], axis=0))
            rows = pl.ds(pl.multiple_of(b * (seg // 2), seg // 2), seg // 2)

            def project(cols):
                qkv = rest(cols)
                return jnp.concatenate(
                    [qkv[:2 * n_mem], _unpack(early_ref[rows, cols]), qkv[2 * n_mem:]], axis=0)
        else:
            project = projector(h_ref[...])
        mems = mix(project, [b + _LAG, n_seg + b], ffn_blocks)
        h_ref[:2 * n_mem, :] = mems.astype(jnp.bfloat16)
        h_ref[2 * n_mem:, :] = h_next
        return mems[n_mem:]

    x_copy = pltpu.make_async_copy(xt_hbm, xt_ref, sem.at[0])
    head_copies = [
        [pltpu.make_async_copy(w.bitcast(jnp.uint32).at[:, p, :], stage_ref.at[i, p],
                               stage_sem.at[i * n_pairs + p])
         for i, w in enumerate((wq_hbm, wk_hbm, wv_hbm))]
        for p in range(n_pairs)]
    wo_copies = [
        pltpu.make_async_copy(wot_hbm.bitcast(jnp.uint32).at[h],
                              wot_ref.at[:, pl.ds(h * d_head, d_head)], wo_sem.at[h])
        for h in range(n_heads)]
    ffn_copies = [
        pltpu.make_async_copy(src.bitcast(jnp.uint32), dst, sem.at[1 + i])
        for i, (src, dst) in enumerate(
            ((w1_hbm, w1_ref), (w3_hbm, w3_ref), (w2t_hbm, w2t_ref)))]
    out_copies = [
        pltpu.make_async_copy(xt_ref.at[:, pl.ds(i * _LANES, _LANES)],
                              outt_hbm.at[:, pl.ds(i * _LANES, _LANES)], out_sem.at[i])
        for i in range(n_io)]

    x_copy.start()
    for c in sum(head_copies[:_COPIES_AHEAD], []):
        c.start()
    x_copy.wait()
    for i in range(n_io):
        cols = slice(i * _LANES, (i + 1) * _LANES)
        res_ref[cols, :] = xt_ref[:, cols].astype(jnp.float32).T
    h_early = _layernorm(res_ref[_LAG * seg:(_LAG + _EARLY) * seg, :]).astype(jnp.bfloat16)
    for p in range(n_pairs):
        if p + _COPIES_AHEAD < n_pairs:
            for c in head_copies[p + _COPIES_AHEAD]:
                c.start()
        elif p + _COPIES_AHEAD == n_pairs:
            for c in wo_copies:
                c.start()
        if p == n_pairs - _FFN_COPY_LEAD:
            for c in ffn_copies:
                c.start()
        for i in range(3):
            head_copies[p][i].wait()
            words = stage_ref[i, p]
            lo = pltpu.bitcast(words << 16, jnp.float32)
            hi = pltpu.bitcast(words & jnp.uint32(0xFFFF0000), jnp.float32)
            for half, w in enumerate((lo, hi)):
                col = (3 * (2 * p + half) + i) * d_head
                wqkv_ref[:, col:col + d_head] = _pack(w.astype(jnp.bfloat16))
        cols = slice(6 * p * d_head, 6 * (p + 1) * d_head)
        early_ref[:, cols] = _pack(projector(h_early)(cols))
    for c in wo_copies:
        c.wait()

    mem0 = mem0_ref[...].astype(jnp.float32)
    mem1 = jax.lax.fori_loop(0, _LAG, single_step, mem0)
    for c in ffn_copies:
        c.wait()
    ffn_step([0, 1])
    h_ref[:2 * n_mem, :] = jnp.concatenate([mem1, mem0], axis=0).astype(jnp.bfloat16)
    h_ref[2 * n_mem:, :] = normed([_LAG, n_seg])
    jax.lax.fori_loop(0, _EARLY, functools.partial(double_step, early=True), mem0)
    mem2 = jax.lax.fori_loop(_EARLY, n_seg - _LAG, functools.partial(double_step, early=False),
                             mem0)

    def write_out(first, last):
        for i in range(first, last):
            rows = pl.ds(2 * n_tok + i * _LANES, _LANES)
            xt_ref[:, i * _LANES:(i + 1) * _LANES] = res_ref[rows, :].T.astype(xt_ref.dtype)
        for i in range(first, last):
            out_copies[i].start()

    def tail_step(i, mem):
        r = 2 * n_seg - _LAG + 2 * i
        mem = single_step(r, mem, [jnp.where(i == 0, n_seg - 1, r - 2), r - 1])
        return single_step(r + 1, mem)

    n_done = (n_seg - _LAG - 1) * seg // _LANES
    write_out(0, n_done)
    jax.lax.fori_loop(0, _LAG // 2, tail_step, mem2)
    ffn_step([2 * n_seg - 2, 2 * n_seg - 1])
    write_out(n_done, n_io)
    for c in out_copies:
        c.wait()


@functools.partial(jax.jit, static_argnames=("A_seg_len",))
def pallas_interleave_layers__memory_aug_recurrent_mem_tr__glu_gated_swiglu__prompt_kernel(
    A_x: jax.Array,
    A_mem0: jax.Array,
    A_Wq: jax.Array,
    A_Wk: jax.Array,
    A_Wv: jax.Array,
    A_Wo: jax.Array,
    A_seg_len: int,
    B_x: jax.Array,
    B_w1: jax.Array,
    B_w3: jax.Array,
    B_w2: jax.Array,
):
    del B_x
    _, n_tok, d_model = A_x.shape
    n_mem = A_mem0.shape[1]
    _, n_heads, d_head = A_Wq.shape
    d_ff = B_w1.shape[1]
    bf16 = jnp.bfloat16
    hbm = pl.BlockSpec(memory_space=pltpu.HBM)
    out_t = pl.pallas_call(
        functools.partial(_kernel, seg=A_seg_len),
        out_shape=jax.ShapeDtypeStruct((d_model, n_tok), A_x.dtype),
        in_specs=[hbm, pl.BlockSpec(memory_space=pltpu.VMEM)] + [hbm] * 7,
        out_specs=hbm,
        scratch_shapes=[
            pltpu.VMEM((d_model, n_tok), A_x.dtype),
            pltpu.VMEM((3 * n_tok, d_model), jnp.float32),
            pltpu.VMEM((2 * (n_mem + A_seg_len), d_model), bf16),
            pltpu.VMEM((_EARLY * A_seg_len // 2, 3 * n_heads * d_head), jnp.uint32),
            pltpu.VMEM((3, n_heads // 2, d_model, d_head), jnp.uint32),
            pltpu.VMEM((d_model // 2, 3 * n_heads * d_head), jnp.uint32),
            pltpu.VMEM((d_model // 2, n_heads * d_head), jnp.uint32),
            pltpu.VMEM((d_model // 2, d_ff), jnp.uint32),
            pltpu.VMEM((d_model // 2, d_ff), jnp.uint32),
            pltpu.VMEM((d_model // 2, d_ff), jnp.uint32),
            pltpu.SemaphoreType.DMA((3 * n_heads // 2,)),
            pltpu.SemaphoreType.DMA((n_heads,)),
            pltpu.SemaphoreType.DMA((n_tok // _LANES,)),
            pltpu.SemaphoreType.DMA((4,)),
        ],
        compiler_params=pltpu.CompilerParams(vmem_limit_bytes=110 * 1024 * 1024),
    )(A_x.reshape(n_tok, d_model).T, A_mem0.reshape(n_mem, d_model), A_Wq, A_Wk, A_Wv,
      A_Wo.transpose(0, 2, 1), B_w1, B_w3, B_w2.T)
    return out_t.T.reshape(A_x.shape)
```

```python
import functools
import math

import jax
import jax.numpy as jnp
import jax.experimental.pallas as pl
import jax.experimental.pallas.tpu as pltpu

_EPS = 1e-05
_MASKED = -1000000000.0
_LOG2E = math.log2(math.e)
_LANES = 128
_LAG = 4
_EARLY = 10
_HEADS_PER_GROUP = 4
_FFN_CHUNK = 512
_COPIES_AHEAD = 2
_FFN_COPY_LEAD = 1
_PIPELINE = (("P", 2), ("S", 1), ("X", 1), ("V", 0), ("G", 0), ("O", -1))
_MAX_SKEW = 4


def _layernorm(x):
    m = jnp.mean(x, axis=-1, keepdims=True)
    d = x - m
    v = jnp.mean(d * d, axis=-1, keepdims=True)
    return d * jax.lax.rsqrt(v + _EPS)


def _dot(a, b):
    return jnp.dot(a, b, preferred_element_type=jnp.float32)


def _dot_nt(a, b):
    return jax.lax.dot_general(a, b, (((1,), (1,)), ((), ())),
                               preferred_element_type=jnp.float32)


def _pack(x):
    return pltpu.bitcast(x, jnp.uint32)


def _unpack(words):
    return pltpu.bitcast(words, jnp.bfloat16)


def _attention_masks(n_layers, n_mem, seg):
    rows = n_layers * (n_mem + seg)
    i = jax.lax.broadcasted_iota(jnp.int32, (rows, rows), 0)
    j = jax.lax.broadcasted_iota(jnp.int32, (rows, rows), 1)
    visible = (i < n_layers * n_mem) | (i >= j)
    if n_layers == 1:
        return visible, _MASKED * _LOG2E

    def second_layer(r):
        return ((r >= n_mem) & (r < 2 * n_mem)) | (r >= 2 * n_mem + seg)

    same = second_layer(i) == second_layer(j)
    fill = jnp.where(same, _MASKED * _LOG2E, -jnp.inf).astype(jnp.float32)
    return same & visible, fill


def _kernel(xt_hbm, mem0_ref, wq_hbm, wk_hbm, wv_hbm, wot_hbm, w1_hbm, w3_hbm, w2t_hbm,
            outt_hbm, xt_ref, outt_ref, res_ref, h_ref, early_ref, stage_ref, wqkv_ref, wot_ref, w1_ref,
            w3_ref, w2t_ref, stage_sem, wo_sem, out_sem, sem, *, seg):
    d_model, n_tok = xt_ref.shape
    n_mem = mem0_ref.shape[0]
    n_pairs, _, d_head = stage_ref.shape[1:]
    n_heads = 2 * n_pairs
    n_groups = n_heads // _HEADS_PER_GROUP
    group_cols = 3 * d_head * _HEADS_PER_GROUP
    n_chunks = w1_ref.shape[1] // _FFN_CHUNK
    n_seg = n_tok // seg
    n_io = n_tok // _LANES
    score_scale = d_head ** -0.5 * _LOG2E

    def block(r):
        return pl.ds(pl.multiple_of(r * seg, seg), seg)

    def load_blocks(blocks):
        return jnp.concatenate([res_ref[block(r), :] for r in blocks], axis=0)

    def store_blocks(blocks, value):
        for i, r in enumerate(blocks):
            res_ref[block(r), :] = value[i * seg:(i + 1) * seg]

    def normed(blocks):
        return _layernorm(load_blocks(blocks)).astype(jnp.bfloat16)

    def transpose_out(i):
        rows = pl.ds(pl.multiple_of(2 * n_tok + i * _LANES, _LANES), _LANES)
        outt_ref[i] = res_ref[rows, :].T.astype(outt_ref.dtype)

    def mix(project, attn_blocks, ffn_blocks):
        n_layers = len(attn_blocks)
        if attn_blocks:
            visible, fill = _attention_masks(n_layers, n_mem, seg)
        if ffn_blocks:
            y = load_blocks(ffn_blocks)
            hn = _layernorm(y).astype(jnp.bfloat16)
        qkv, scores, probs, heads, acts, out = {}, {}, {}, {}, [], None

        def part(g, head, which):
            col = (3 * head + which) * d_head
            return qkv[g][:, col:col + d_head]

        for it in range(-_MAX_SKEW, max(n_groups, n_chunks) + _MAX_SKEW):
            for stage, skew in _PIPELINE:
                g = it + skew
                if stage == "G":
                    if ffn_blocks and 0 <= g < n_chunks:
                        cols = slice(g * _FFN_CHUNK, (g + 1) * _FFN_CHUNK)
                        gate = _dot(hn, _unpack(w1_ref[:, cols]))
                        up = _dot(hn, _unpack(w3_ref[:, cols]))
                        acts.append((gate * jax.nn.sigmoid(gate) * up).astype(jnp.bfloat16))
                elif not (attn_blocks and 0 <= g < n_groups):
                    continue
                elif stage == "P":
                    qkv[g] = project(slice(g * group_cols, (g + 1) * group_cols))
                elif stage == "S":
                    scores[g] = [_dot_nt(part(g, i, 0), part(g, i, 1))
                                 for i in range(_HEADS_PER_GROUP)]
                elif stage == "X":
                    probs[g] = []
                    for s in scores[g]:
                        s = jnp.where(visible, s * score_scale, fill)
                        p = jnp.exp2(s - jnp.max(s, axis=-1, keepdims=True))
                        inv = 1.0 / jnp.sum(p, axis=-1, keepdims=True)
                        probs[g].append((p.astype(jnp.bfloat16), inv))
                elif stage == "V":
                    heads[g] = [(_dot(p, part(g, i, 2)) * inv).astype(jnp.bfloat16)
                                for i, (p, inv) in enumerate(probs[g])]
                elif stage == "O":
                    width = _HEADS_PER_GROUP * d_head
                    o = _dot_nt(jnp.concatenate(heads[g], axis=1),
                                _unpack(wot_ref[:, g * width:(g + 1) * width]))
                    out = o if out is None else out + o
        mems = xa = None
        if ffn_blocks:
            y = y + _dot_nt(jnp.concatenate(acts, axis=1), _unpack(w2t_ref[...]))
        if attn_blocks:
            mems = out[:n_layers * n_mem]
            xa = load_blocks(attn_blocks) + out[n_layers * n_mem:]
            store_blocks(attn_blocks, xa)
        if ffn_blocks:
            store_blocks([r + n_seg for r in ffn_blocks], y)
        return mems

    def projector(h):
        return lambda cols: _dot(h, _unpack(wqkv_ref[:, cols])).astype(jnp.bfloat16)

    def single_step(r, mem, ffn_blocks=()):
        h = jnp.concatenate([mem, _layernorm(load_blocks([r]))], axis=0)
        return mix(projector(h.astype(jnp.bfloat16)), [r], ffn_blocks)

    def ffn_step(blocks):
        mix(None, [], blocks)

    def double_step(b, _, *, early):
        ffn_blocks = [jnp.where(b == 0, _LAG - 2, b + _LAG - 1),
                      jnp.where(b == 0, _LAG - 1, n_seg + b - 1)]
        h_next = normed([jnp.minimum(b + 1 + _LAG, n_seg - 1), n_seg + b + 1])
        if early:
            rest = projector(jnp.concatenate(
                [h_ref[:2 * n_mem, :], h_ref[2 * n_mem + seg:, :]], axis=0))
            rows = pl.ds(pl.multiple_of(b * (seg // 2), seg // 2), seg // 2)

            def project(cols):
                qkv = rest(cols)
                return jnp.concatenate(
                    [qkv[:2 * n_mem], _unpack(early_ref[rows, cols]), qkv[2 * n_mem:]], axis=0)
        else:
            project = projector(h_ref[...])
            transpose_out((b - 5) * seg // _LANES)
        mems = mix(project, [b + _LAG, n_seg + b], ffn_blocks)
        h_ref[:2 * n_mem, :] = mems.astype(jnp.bfloat16)
        h_ref[2 * n_mem:, :] = h_next
        return mems[n_mem:]

    n_first = pl.cdiv((_LAG + _EARLY) * seg, _LANES)
    x_copies = [
        pltpu.make_async_copy(xt_hbm.at[:, cols], xt_ref.at[:, cols], sem.at[i])
        for i, cols in enumerate((pl.ds(0, n_first * _LANES),
                                  pl.ds(n_first * _LANES, n_tok - n_first * _LANES)))]
    head_copies = [
        [pltpu.make_async_copy(w.bitcast(jnp.uint32).at[:, p, :], stage_ref.at[i, p],
                               stage_sem.at[i * n_pairs + p])
         for i, w in enumerate((wq_hbm, wk_hbm, wv_hbm))]
        for p in range(n_pairs)]
    wo_copies = [
        pltpu.make_async_copy(wot_hbm.bitcast(jnp.uint32).at[h],
                              wot_ref.at[:, pl.ds(h * d_head, d_head)], wo_sem.at[h])
        for h in range(n_heads)]
    ffn_copies = [
        pltpu.make_async_copy(src.bitcast(jnp.uint32), dst, sem.at[2 + i])
        for i, (src, dst) in enumerate(
            ((w1_hbm, w1_ref), (w3_hbm, w3_ref), (w2t_hbm, w2t_ref)))]
    out_copies = [
        pltpu.make_async_copy(outt_ref.at[i],
                              outt_hbm.at[:, pl.ds(i * _LANES, _LANES)], out_sem.at[i])
        for i in range(n_io)]

    def transpose_x(i):
        cols = slice(i * _LANES, (i + 1) * _LANES)
        res_ref[cols, :] = xt_ref[:, cols].astype(jnp.float32).T

    pairs = _HEADS_PER_GROUP // 2
    group_copies = [sum(head_copies[g * pairs:(g + 1) * pairs], []) for g in range(n_groups)]
    x_copies[0].start()
    for c in sum(group_copies[:_COPIES_AHEAD], []):
        c.start()
    x_copies[1].start()
    x_copies[0].wait()
    for i in range(n_first):
        transpose_x(i)
    h_early = normed(range(_LAG, _LAG + _EARLY))
    late_x = list(range(n_first, n_io))
    for g in range(n_groups):
        if g + _COPIES_AHEAD < n_groups:
            for c in group_copies[g + _COPIES_AHEAD]:
                c.start()
        elif g + _COPIES_AHEAD == n_groups:
            for c in wo_copies:
                c.start()
        if g == n_groups - _FFN_COPY_LEAD:
            for c in ffn_copies:
                c.start()
        if g == n_groups // 2:
            x_copies[1].wait()
        for c in group_copies[g]:
            c.wait()
        for p in range(g * pairs, (g + 1) * pairs):
            for i in range(3):
                words = stage_ref[i, p]
                lo = pltpu.bitcast(words << 16, jnp.float32)
                hi = pltpu.bitcast(words & jnp.uint32(0xFFFF0000), jnp.float32)
                for half, w in enumerate((lo, hi)):
                    col = (3 * (2 * p + half) + i) * d_head
                    wqkv_ref[:, col:col + d_head] = _pack(w.astype(jnp.bfloat16))
        cols = slice(g * group_cols, (g + 1) * group_cols)
        early_ref[:, cols] = _pack(projector(h_early)(cols))
        if g >= n_groups // 2:
            for i in late_x[g - n_groups // 2::n_groups - n_groups // 2]:
                transpose_x(i)
    for c in wo_copies:
        c.wait()

    mem0 = mem0_ref[...].astype(jnp.float32)
    mem1 = jax.lax.fori_loop(0, _LAG, single_step, mem0)
    for c in ffn_copies:
        c.wait()
    ffn_step([0, 1])
    h_ref[:2 * n_mem, :] = jnp.concatenate([mem1, mem0], axis=0).astype(jnp.bfloat16)
    h_ref[2 * n_mem:, :] = normed([_LAG, n_seg])
    jax.lax.fori_loop(0, _EARLY, functools.partial(double_step, early=True), mem0)
    mem2 = jax.lax.fori_loop(_EARLY, n_seg - _LAG, functools.partial(double_step, early=False),
                             mem0)

    def tail_step(i, mem):
        r = 2 * n_seg - _LAG + 2 * i
        mem = single_step(r, mem, [jnp.where(i == 0, n_seg - 1, r - 2), r - 1])
        return single_step(r + 1, mem)

    n_done = (n_seg - _LAG - 6) * seg // _LANES + 1
    for i in range((_EARLY - 5) * seg // _LANES):
        transpose_out(i)
    for c in out_copies[:n_done]:
        c.start()
    jax.lax.fori_loop(0, _LAG // 2, tail_step, mem2)
    ffn_step([2 * n_seg - 2, 2 * n_seg - 1])
    for i in range(n_done, n_io):
        transpose_out(i)
        out_copies[i].start()
    for c in out_copies:
        c.wait()


@functools.partial(jax.jit, static_argnames=("A_seg_len",))
def pallas_interleave_layers__memory_aug_recurrent_mem_tr__glu_gated_swiglu__prompt_kernel(
    A_x: jax.Array,
    A_mem0: jax.Array,
    A_Wq: jax.Array,
    A_Wk: jax.Array,
    A_Wv: jax.Array,
    A_Wo: jax.Array,
    A_seg_len: int,
    B_x: jax.Array,
    B_w1: jax.Array,
    B_w3: jax.Array,
    B_w2: jax.Array,
):
    del B_x
    _, n_tok, d_model = A_x.shape
    n_mem = A_mem0.shape[1]
    _, n_heads, d_head = A_Wq.shape
    d_ff = B_w1.shape[1]
    bf16 = jnp.bfloat16
    hbm = pl.BlockSpec(memory_space=pltpu.HBM)
    out_t = pl.pallas_call(
        functools.partial(_kernel, seg=A_seg_len),
        out_shape=jax.ShapeDtypeStruct((d_model, n_tok), A_x.dtype),
        in_specs=[hbm, pl.BlockSpec(memory_space=pltpu.VMEM)] + [hbm] * 7,
        out_specs=hbm,
        scratch_shapes=[
            pltpu.VMEM((d_model, n_tok), A_x.dtype),
            pltpu.VMEM((n_tok // _LANES, d_model, _LANES), A_x.dtype),
            pltpu.VMEM((3 * n_tok, d_model), jnp.float32),
            pltpu.VMEM((2 * (n_mem + A_seg_len), d_model), bf16),
            pltpu.VMEM((_EARLY * A_seg_len // 2, 3 * n_heads * d_head), jnp.uint32),
            pltpu.VMEM((3, n_heads // 2, d_model, d_head), jnp.uint32),
            pltpu.VMEM((d_model // 2, 3 * n_heads * d_head), jnp.uint32),
            pltpu.VMEM((d_model // 2, n_heads * d_head), jnp.uint32),
            pltpu.VMEM((d_model // 2, d_ff), jnp.uint32),
            pltpu.VMEM((d_model // 2, d_ff), jnp.uint32),
            pltpu.VMEM((d_model // 2, d_ff), jnp.uint32),
            pltpu.SemaphoreType.DMA((3 * n_heads // 2,)),
            pltpu.SemaphoreType.DMA((n_heads,)),
            pltpu.SemaphoreType.DMA((n_tok // _LANES,)),
            pltpu.SemaphoreType.DMA((5,)),
        ],
        compiler_params=pltpu.CompilerParams(vmem_limit_bytes=110 * 1024 * 1024),
    )(A_x.reshape(n_tok, d_model).T, A_mem0.reshape(n_mem, d_model), A_Wq, A_Wk, A_Wv,
      A_Wo.transpose(0, 2, 1), B_w1, B_w3, B_w2.T)
    return out_t.T.reshape(A_x.shape)
```

```python
import functools
import math

import jax
import jax.numpy as jnp
import jax.experimental.pallas as pl
import jax.experimental.pallas.tpu as pltpu

_EPS = 1e-05
_MASKED = -1000000000.0
_LOG2E = math.log2(math.e)
_LANES = 128
_LAG = 6
_EARLY = 8
_HEADS_PER_GROUP = 4
_FFN_CHUNK = 256
_COPIES_AHEAD = 2
_FFN_COPY_LEAD = 2
_STAGE_ORDER = [(t[0], int(t[1:])) for t in (
    "P0 G0 P1 S0 G1 P2 S1 V0 G2 G3 P3 V1 G4 O0 S2 P4 V2 G5 O1 S3 P5 S4 V3 O2 G6 V4 G7 S5 "
    "P6 O3 S6 V5 P7 G8 S7 O4 V6 D0 O5 V7 O6 O7").split()]


def _layernorm(x):
    m = jnp.mean(x, axis=-1, keepdims=True)
    d = x - m
    v = jnp.mean(d * d, axis=-1, keepdims=True)
    return d * jax.lax.rsqrt(v + _EPS)


def _dot(a, b):
    return jnp.dot(a, b, preferred_element_type=jnp.float32)


def _dot_nt(a, b):
    return jax.lax.dot_general(a, b, (((1,), (1,)), ((), ())),
                               preferred_element_type=jnp.float32)


def _pack(x):
    return pltpu.bitcast(x, jnp.uint32)


def _unpack(words):
    return pltpu.bitcast(words, jnp.bfloat16)


def _attention_masks(n_layers, n_mem, seg):
    rows = n_layers * (n_mem + seg)
    i = jax.lax.broadcasted_iota(jnp.int32, (rows, rows), 0)
    j = jax.lax.broadcasted_iota(jnp.int32, (rows, rows), 1)
    visible = (i < n_layers * n_mem) | (i >= j)
    if n_layers == 1:
        return visible, _MASKED * _LOG2E

    def second_layer(r):
        return ((r >= n_mem) & (r < 2 * n_mem)) | (r >= 2 * n_mem + seg)

    same = second_layer(i) == second_layer(j)
    fill = jnp.where(same, _MASKED * _LOG2E, -jnp.inf).astype(jnp.float32)
    return same & visible, fill


def _kernel(xt_hbm, mem0_ref, wq_hbm, wk_hbm, wv_hbm, wot_hbm, w1_hbm, w3_hbm, w2t_hbm,
            outt_hbm, xt_ref, outt_ref, res_ref, h_ref, early_ref, stage_ref, wqkv_ref, wot_ref, w13_ref,
            w2t_ref, stage_sem, wo_sem, ffn_sem, out_sem, sem, *, seg):
    d_model, n_tok = xt_ref.shape
    n_mem = mem0_ref.shape[0]
    n_pairs, _, d_head = stage_ref.shape[1:]
    n_heads = 2 * n_pairs
    n_groups = n_heads // _HEADS_PER_GROUP
    group_cols = 3 * d_head * _HEADS_PER_GROUP
    half_ff = w2t_ref.shape[2]
    n_chunks = half_ff // _FFN_CHUNK
    n_seg = n_tok // seg
    n_io = n_tok // _LANES
    score_scale = d_head ** -0.5 * _LOG2E

    def block(r):
        return pl.ds(pl.multiple_of(r * seg, seg), seg)

    def load_blocks(blocks):
        return jnp.concatenate([res_ref[block(r), :] for r in blocks], axis=0)

    def store_blocks(blocks, value):
        for i, r in enumerate(blocks):
            res_ref[block(r), :] = value[i * seg:(i + 1) * seg]

    def normed(blocks):
        return _layernorm(load_blocks(blocks)).astype(jnp.bfloat16)

    def transpose_out(i):
        rows = pl.ds(pl.multiple_of(2 * n_tok + i * _LANES, _LANES), _LANES)
        outt_ref[i] = res_ref[rows, :].T.astype(outt_ref.dtype)

    def gated(hn, half, c):
        cols = slice(2 * c * _FFN_CHUNK, 2 * (c + 1) * _FFN_CHUNK)
        both = _dot(hn, _unpack(w13_ref[half, :, cols]))
        gate, up = both[:, :_FFN_CHUNK], both[:, _FFN_CHUNK:]
        return (gate * jax.nn.sigmoid(gate) * up).astype(jnp.bfloat16)

    def mix(project, attn_blocks, ffn_blocks, half):
        n_layers = len(attn_blocks)
        visible, fill = _attention_masks(n_layers, n_mem, seg)
        if ffn_blocks:
            hn = normed(ffn_blocks)
        qkv, probs, heads, acts, out = {}, {}, {}, [], None

        def part(g, head, which):
            col = (3 * head + which) * d_head
            return qkv[g][:, col:col + d_head]

        for stage, g in _STAGE_ORDER:
            if stage in "GD" and not ffn_blocks:
                continue
            if stage == "P":
                qkv[g] = project(slice(g * group_cols, (g + 1) * group_cols))
            elif stage == "S":
                probs[g] = []
                for s in [_dot_nt(part(g, i, 0), part(g, i, 1)) for i in range(_HEADS_PER_GROUP)]:
                    s = jnp.where(visible, s * score_scale, fill)
                    p = jnp.exp2(s - jnp.max(s, axis=-1, keepdims=True))
                    inv = 1.0 / jnp.sum(p, axis=-1, keepdims=True)
                    probs[g].append((p.astype(jnp.bfloat16), inv))
            elif stage == "V":
                heads[g] = [(_dot(p, part(g, i, 2)) * inv).astype(jnp.bfloat16)
                            for i, (p, inv) in enumerate(probs[g])]
            elif stage == "O":
                width = _HEADS_PER_GROUP * d_head
                o = _dot_nt(jnp.concatenate(heads[g], axis=1),
                            _unpack(wot_ref[:, g * width:(g + 1) * width]))
                out = o if out is None else out + o
            elif stage == "G":
                acts.append(gated(hn, half, g))
            elif stage == "D":
                y = _dot_nt(_unpack(w2t_ref[half]), jnp.concatenate(acts, axis=1)).T
                y = y + load_blocks([r + half * n_seg for r in ffn_blocks])
        store_blocks(attn_blocks, load_blocks(attn_blocks) + out[n_layers * n_mem:])
        if ffn_blocks:
            store_blocks([r + n_seg for r in ffn_blocks], y)
        return out[:n_layers * n_mem]

    def projector(h):
        return lambda cols: _dot(h, _unpack(wqkv_ref[:, cols])).astype(jnp.bfloat16)

    def single_step(r, mem, ffn_blocks=(), half=None):
        h = jnp.concatenate([mem, _layernorm(load_blocks([r]))], axis=0)
        return mix(projector(h.astype(jnp.bfloat16)), [r], ffn_blocks, half)

    def ffn_step(blocks):
        y = load_blocks(blocks)
        hn = _layernorm(y).astype(jnp.bfloat16)
        for half in range(2):
            acts = jnp.concatenate([gated(hn, half, c) for c in range(n_chunks)], axis=1)
            y = y + _dot_nt(acts, _unpack(w2t_ref[half]))
        store_blocks([r + n_seg for r in blocks], y)

    def double_step(b, _, *, early):
        half = b % 2
        first = b - half
        f1 = jnp.where(first == 0, _LAG - 4, first + _LAG - 2)
        f2 = jnp.where(first == 0, _LAG - 2, n_seg + first - 2)
        h_next = normed([jnp.minimum(b + 1 + _LAG, n_seg - 1), n_seg + b + 1])
        if early:
            @pl.when(b == 2)
            def _refresh():
                h_ref[2 * n_mem + seg:, :] = normed([n_seg + 2])

            rest = projector(jnp.concatenate(
                [h_ref[:2 * n_mem, :], h_ref[2 * n_mem + seg:, :]], axis=0))
            rows = pl.ds(pl.multiple_of(b * (seg // 2), seg // 2), seg // 2)

            def project(cols):
                qkv = rest(cols)
                return jnp.concatenate(
                    [qkv[:2 * n_mem], _unpack(early_ref[rows, cols]), qkv[2 * n_mem:]], axis=0)
        else:
            project = projector(h_ref[...])
            transpose_out((b - 7) * seg // _LANES)
        mems = mix(project, [b + _LAG, n_seg + b], [f1, f1 + 1, f2, f2 + 1], half)
        h_ref[:2 * n_mem, :] = mems.astype(jnp.bfloat16)
        h_ref[2 * n_mem:, :] = h_next
        return mems[n_mem:]

    n_first = pl.cdiv((_LAG + _EARLY) * seg, _LANES)
    x_copies = [
        pltpu.make_async_copy(xt_hbm.at[:, cols], xt_ref.at[:, cols], sem.at[i])
        for i, cols in enumerate((pl.ds(0, n_first * _LANES),
                                  pl.ds(n_first * _LANES, n_tok - n_first * _LANES)))]
    head_copies = [
        [pltpu.make_async_copy(w.bitcast(jnp.uint32).at[:, p, :], stage_ref.at[i, p],
                               stage_sem.at[i * n_pairs + p])
         for i, w in enumerate((wq_hbm, wk_hbm, wv_hbm))]
        for p in range(n_pairs)]
    wo_copies = [
        pltpu.make_async_copy(wot_hbm.bitcast(jnp.uint32).at[h],
                              wot_ref.at[:, pl.ds(h * d_head, d_head)], wo_sem.at[h])
        for h in range(n_heads)]
    ffn_pieces = [(w2t_hbm, half * half_ff, half_ff, w2t_ref.at[half]) for half in range(2)]
    for half in range(2):
        for c in range(n_chunks):
            for i, w in enumerate((w1_hbm, w3_hbm)):
                dst = w13_ref.at[half, :, pl.ds((2 * c + i) * _FFN_CHUNK, _FFN_CHUNK)]
                ffn_pieces.append((w, half * half_ff + c * _FFN_CHUNK, _FFN_CHUNK, dst))
    ffn_copies = [
        pltpu.make_async_copy(w.bitcast(jnp.uint32).at[:, pl.ds(col, width)], dst, ffn_sem.at[i])
        for i, (w, col, width, dst) in enumerate(ffn_pieces)]
    out_copies = [
        pltpu.make_async_copy(outt_ref.at[i],
                              outt_hbm.at[:, pl.ds(i * _LANES, _LANES)], out_sem.at[i])
        for i in range(n_io)]

    def transpose_x(i):
        cols = slice(i * _LANES, (i + 1) * _LANES)
        res_ref[cols, :] = xt_ref[:, cols].astype(jnp.float32).T

    pairs = _HEADS_PER_GROUP // 2
    group_copies = [sum(head_copies[g * pairs:(g + 1) * pairs], []) for g in range(n_groups)]
    x_copies[0].start()
    for c in sum(group_copies[:_COPIES_AHEAD], []):
        c.start()
    x_copies[1].start()
    x_copies[0].wait()
    for i in range(n_first):
        transpose_x(i)
    h_early = normed(range(_LAG, _LAG + _EARLY))
    late_x = list(range(n_first, n_io))
    for g in range(n_groups):
        if g + _COPIES_AHEAD < n_groups:
            for c in group_copies[g + _COPIES_AHEAD]:
                c.start()
        elif g + _COPIES_AHEAD == n_groups:
            for c in wo_copies:
                c.start()
        if g == n_groups - _FFN_COPY_LEAD:
            for c in ffn_copies:
                c.start()
        if g == n_groups // 2:
            x_copies[1].wait()
        for c in group_copies[g]:
            c.wait()
        for p in range(g * pairs, (g + 1) * pairs):
            for i in range(3):
                words = stage_ref[i, p]
                lo = pltpu.bitcast(words << 16, jnp.float32)
                hi = pltpu.bitcast(words & jnp.uint32(0xFFFF0000), jnp.float32)
                for half, w in enumerate((lo, hi)):
                    col = (3 * (2 * p + half) + i) * d_head
                    wqkv_ref[:, col:col + d_head] = _pack(w.astype(jnp.bfloat16))
        cols = slice(g * group_cols, (g + 1) * group_cols)
        early_ref[:, cols] = _pack(projector(h_early)(cols))
        if g >= n_groups // 2:
            for i in late_x[g - n_groups // 2::n_groups - n_groups // 2]:
                transpose_x(i)
    for c in wo_copies:
        c.wait()

    mem0 = mem0_ref[...].astype(jnp.float32)
    mem1 = jax.lax.fori_loop(0, _LAG, single_step, mem0)
    for c in ffn_copies:
        c.wait()
    ffn_step([0, 1])
    h_ref[:2 * n_mem, :] = jnp.concatenate([mem1, mem0], axis=0).astype(jnp.bfloat16)
    h_ref[2 * n_mem:, :] = normed([_LAG, n_seg])
    jax.lax.fori_loop(0, _EARLY, functools.partial(double_step, early=True), mem0)
    mem2 = jax.lax.fori_loop(_EARLY, n_seg - _LAG, functools.partial(double_step, early=False),
                             mem0)

    def tail_step(i, mem):
        r = 2 * n_seg - _LAG + i
        f1 = jnp.where(i < 2, n_seg - 2, 2 * n_seg - 6)
        f2 = jnp.where(i < 2, 2 * n_seg - 8, 2 * n_seg - 4)
        return jax.lax.cond(
            i // 2 == 1,
            lambda: single_step(r, mem),
            lambda: single_step(r, mem, [f1, f1 + 1, f2, f2 + 1], i % 2))

    n_done = (n_seg - _LAG - 8) * seg // _LANES + 1
    for i in range((_EARLY - 7) * seg // _LANES):
        transpose_out(i)
    for c in out_copies[:n_done]:
        c.start()
    jax.lax.fori_loop(0, _LAG, tail_step, mem2)
    ffn_step([2 * n_seg - 2, 2 * n_seg - 1])
    for i in range(n_done, n_io):
        transpose_out(i)
        out_copies[i].start()
    for c in out_copies:
        c.wait()


@functools.partial(jax.jit, static_argnames=("A_seg_len",))
def pallas_interleave_layers__memory_aug_recurrent_mem_tr__glu_gated_swiglu__prompt_kernel(
    A_x: jax.Array,
    A_mem0: jax.Array,
    A_Wq: jax.Array,
    A_Wk: jax.Array,
    A_Wv: jax.Array,
    A_Wo: jax.Array,
    A_seg_len: int,
    B_x: jax.Array,
    B_w1: jax.Array,
    B_w3: jax.Array,
    B_w2: jax.Array,
):
    del B_x
    _, n_tok, d_model = A_x.shape
    n_mem = A_mem0.shape[1]
    _, n_heads, d_head = A_Wq.shape
    d_ff = B_w1.shape[1]
    bf16 = jnp.bfloat16
    hbm = pl.BlockSpec(memory_space=pltpu.HBM)
    out_t = pl.pallas_call(
        functools.partial(_kernel, seg=A_seg_len),
        out_shape=jax.ShapeDtypeStruct((d_model, n_tok), A_x.dtype),
        in_specs=[hbm, pl.BlockSpec(memory_space=pltpu.VMEM)] + [hbm] * 7,
        out_specs=hbm,
        scratch_shapes=[
            pltpu.VMEM((d_model, n_tok), A_x.dtype),
            pltpu.VMEM((n_tok // _LANES, d_model, _LANES), A_x.dtype),
            pltpu.VMEM((3 * n_tok, d_model), jnp.float32),
            pltpu.VMEM((2 * (n_mem + A_seg_len), d_model), bf16),
            pltpu.VMEM((_EARLY * A_seg_len // 2, 3 * n_heads * d_head), jnp.uint32),
            pltpu.VMEM((3, n_heads // 2, d_model, d_head), jnp.uint32),
            pltpu.VMEM((d_model // 2, 3 * n_heads * d_head), jnp.uint32),
            pltpu.VMEM((d_model // 2, n_heads * d_head), jnp.uint32),
            pltpu.VMEM((2, d_model // 2, d_ff), jnp.uint32),
            pltpu.VMEM((2, d_model // 2, d_ff // 2), jnp.uint32),
            pltpu.SemaphoreType.DMA((3 * n_heads // 2,)),
            pltpu.SemaphoreType.DMA((n_heads,)),
            pltpu.SemaphoreType.DMA((2 + 2 * d_ff // _FFN_CHUNK,)),
            pltpu.SemaphoreType.DMA((n_tok // _LANES,)),
            pltpu.SemaphoreType.DMA((2,)),
        ],
        compiler_params=pltpu.CompilerParams(vmem_limit_bytes=110 * 1024 * 1024),
    )(A_x.reshape(n_tok, d_model).T, A_mem0.reshape(n_mem, d_model), A_Wq, A_Wk, A_Wv,
      A_Wo.transpose(0, 2, 1), B_w1, B_w3, B_w2.T)
    return out_t.T.reshape(A_x.shape)
```

```python
import functools
import math

import jax
import jax.numpy as jnp
import jax.experimental.pallas as pl
import jax.experimental.pallas.tpu as pltpu

_EPS = 1e-05
_MASKED = -1000000000.0
_LOG2E = math.log2(math.e)
_LANES = 128
_LAG = 4
_EARLY = 12
_HEADS_PER_GROUP = 4
_FFN_CHUNK = 256
_COPIES_AHEAD = 2
_FFN_COPY_LEAD = 2
_STAGE_ORDER = [(t[0], int(t[1:])) for t in (
    "P0 G0 P1 S0 G1 P2 S1 V0 G2 G3 P3 V1 G4 O0 S2 P4 V2 G5 O1 S3 P5 S4 V3 O2 G6 V4 G7 S5 "
    "P6 O3 S6 V5 P7 G8 S7 O4 V6 D0 O5 V7 O6 O7").split()]


def _layernorm(x):
    m = jnp.mean(x, axis=-1, keepdims=True)
    d = x - m
    v = jnp.mean(d * d, axis=-1, keepdims=True)
    return d * jax.lax.rsqrt(v + _EPS)


def _dot(a, b):
    return jnp.dot(a, b, preferred_element_type=jnp.float32)


def _dot_nt(a, b):
    return jax.lax.dot_general(a, b, (((1,), (1,)), ((), ())),
                               preferred_element_type=jnp.float32)


def _pack(x):
    return pltpu.bitcast(x, jnp.uint32)


def _unpack(words):
    return pltpu.bitcast(words, jnp.bfloat16)


def _attention_masks(n_layers, n_mem, seg):
    rows = n_layers * (n_mem + seg)
    i = jax.lax.broadcasted_iota(jnp.int32, (rows, rows), 0)
    j = jax.lax.broadcasted_iota(jnp.int32, (rows, rows), 1)
    visible = (i < n_layers * n_mem) | (i >= j)
    if n_layers == 1:
        return visible, _MASKED * _LOG2E

    def second_layer(r):
        return ((r >= n_mem) & (r < 2 * n_mem)) | (r >= 2 * n_mem + seg)

    same = second_layer(i) == second_layer(j)
    fill = jnp.where(same, _MASKED * _LOG2E, -jnp.inf).astype(jnp.float32)
    return same & visible, fill


def _kernel(xt_hbm, mem0_ref, wq_hbm, wk_hbm, wv_hbm, wot_hbm, w1_hbm, w3_hbm, w2t_hbm,
            outt_hbm, tile_ref, res_ref, h_ref, early_h_ref, early_ref, stage_ref, wqkv_ref, wot_ref, w13_ref,
            w2t_ref, stage_sem, wo_sem, ffn_sem, tile_sem, *, seg):
    d_model, n_tok = xt_hbm.shape
    n_mem = mem0_ref.shape[0]
    _, n_heads, d_head = wq_hbm.shape
    n_groups = n_heads // _HEADS_PER_GROUP
    half_ff = w2t_ref.shape[2]
    n_chunks = half_ff // _FFN_CHUNK
    n_seg = n_tok // seg
    n_io = n_tok // _LANES
    score_scale = d_head ** -0.5 * _LOG2E

    def block(r):
        return pl.ds(pl.multiple_of(r * seg, seg), seg)

    def load_blocks(blocks):
        return jnp.concatenate([res_ref[block(r), :] for r in blocks], axis=0)

    def store_blocks(blocks, value):
        for i, r in enumerate(blocks):
            res_ref[block(r), :] = value[i * seg:(i + 1) * seg]

    def normed(blocks):
        return _layernorm(load_blocks(blocks)).astype(jnp.bfloat16)

    def transpose_out(i):
        rows = pl.ds(pl.multiple_of(2 * n_tok + i * _LANES, _LANES), _LANES)
        tile_ref[i] = res_ref[rows, :].T.astype(tile_ref.dtype)

    def gated(hn, half, c):
        cols = slice(2 * c * _FFN_CHUNK, 2 * (c + 1) * _FFN_CHUNK)
        both = _dot(hn, _unpack(w13_ref[half, :, cols]))
        gate, up = both[:, :_FFN_CHUNK], both[:, _FFN_CHUNK:]
        return (gate * jax.nn.sigmoid(gate) * up).astype(jnp.bfloat16)

    def mix(project, attn_blocks, ffn_blocks, half):
        n_layers = len(attn_blocks)
        if attn_blocks:
            visible, fill = _attention_masks(n_layers, n_mem, seg)
        if ffn_blocks:
            hn = normed(ffn_blocks)
        qkv, probs, heads, acts, out, y = {}, {}, {}, [], None, None

        def part(g, head, which):
            col = (3 * head + which) * d_head
            return qkv[g][:, col:col + d_head]

        for stage, g in _STAGE_ORDER:
            if not (ffn_blocks if stage in "GD" else attn_blocks):
                continue
            if stage == "P":
                qkv[g] = project(g)
            elif stage == "S":
                probs[g] = []
                for s in [_dot_nt(part(g, i, 0), part(g, i, 1)) for i in range(_HEADS_PER_GROUP)]:
                    s = jnp.where(visible, s * score_scale, fill)
                    p = jnp.exp2(s - jnp.max(s, axis=-1, keepdims=True))
                    inv = 1.0 / jnp.sum(p, axis=-1, keepdims=True)
                    probs[g].append((p.astype(jnp.bfloat16), inv))
            elif stage == "V":
                heads[g] = [(_dot(p, part(g, i, 2)) * inv).astype(jnp.bfloat16)
                            for i, (p, inv) in enumerate(probs[g])]
            elif stage == "O":
                width = _HEADS_PER_GROUP * d_head
                o = _dot_nt(jnp.concatenate(heads[g], axis=1),
                            _unpack(wot_ref[:, g * width:(g + 1) * width]))
                out = o if out is None else out + o
            elif stage == "G":
                acts.append(gated(hn, half, g))
            elif stage == "D":
                y = _dot_nt(_unpack(w2t_ref[half]), jnp.concatenate(acts, axis=1)).T
                y = y + load_blocks([r + half * n_seg for r in ffn_blocks])
        if ffn_blocks:
            store_blocks([r + n_seg for r in ffn_blocks], y)
        if attn_blocks:
            store_blocks(attn_blocks, load_blocks(attn_blocks) + out[n_layers * n_mem:])
            return out[:n_layers * n_mem], y

    def projector(h):
        return lambda g: _dot(h, _unpack(wqkv_ref[g])).astype(jnp.bfloat16)

    def single_step(r, mem, ffn_blocks=(), half=None):
        h = jnp.concatenate([mem, _layernorm(load_blocks([r]))], axis=0)
        return mix(projector(h.astype(jnp.bfloat16)), [r], ffn_blocks, half)[0]

    def ffn_only(first):
        @pl.loop(0, 2)
        def _(half):
            mix(None, [], [first + i for i in range(4)], half)

    def double_step(b, _, *, early, with_ffn=True):
        half = b % 2
        f1, f2 = b - half + _LAG - 2, n_seg + b - half - 2
        if early:
            rest = projector(jnp.concatenate(
                [h_ref[:2 * n_mem, :], h_ref[2 * n_mem + seg:, :]], axis=0))
            rows = pl.ds(pl.multiple_of(b * (seg // 2), seg // 2), seg // 2)

            def project(g):
                qkv = rest(g)
                known = _unpack(early_ref[g, rows, :])
                return jnp.concatenate([qkv[:2 * n_mem], known, qkv[2 * n_mem:]], axis=0)
        else:
            project = projector(h_ref[...])
            transpose_out((b - 7) * seg // _LANES)
        h1 = normed([jnp.minimum(b + 1 + _LAG, n_seg - 1)])
        x2 = load_blocks([n_seg + b + 1 - half])
        mems, y = mix(project, [b + _LAG, n_seg + b],
                      [f1, f1 + 1, f2, f2 + 1] if with_ffn else [], half)
        x2 = jnp.where(half == 1, y[:seg], x2) if with_ffn else load_blocks([n_seg + b + 1])
        h_ref[:2 * n_mem, :] = mems.astype(jnp.bfloat16)
        h_ref[2 * n_mem:2 * n_mem + seg, :] = h1
        h_ref[2 * n_mem + seg:, :] = _layernorm(x2).astype(jnp.bfloat16)
        return mems[n_mem:]

    pairs = _HEADS_PER_GROUP // 2

    def head_copies(g):
        return [pltpu.make_async_copy(w.bitcast(jnp.uint32).at[:, g * pairs + p, :],
                                      stage_ref.at[g, 3 * p + i], stage_sem.at[3 * (g * pairs + p) + i])
                for p in range(pairs) for i, w in enumerate((wq_hbm, wk_hbm, wv_hbm))]

    def x_copy(i):
        cols = pl.ds(pl.multiple_of(i * _LANES, _LANES), _LANES)
        return pltpu.make_async_copy(xt_hbm.at[:, cols], tile_ref.at[i], tile_sem.at[i])

    wo_copies = [
        pltpu.make_async_copy(wot_hbm.bitcast(jnp.uint32).at[h],
                              wot_ref.at[:, pl.ds(h * d_head, d_head)], wo_sem.at[h])
        for h in range(n_heads)]
    ffn_pieces = [(w2t_hbm, half * half_ff, half_ff, w2t_ref.at[half]) for half in range(2)]
    for half in range(2):
        for c in range(n_chunks):
            for i, w in enumerate((w1_hbm, w3_hbm)):
                dst = w13_ref.at[half, :, pl.ds((2 * c + i) * _FFN_CHUNK, _FFN_CHUNK)]
                ffn_pieces.append((w, half * half_ff + c * _FFN_CHUNK, _FFN_CHUNK, dst))
    ffn_copies = [
        pltpu.make_async_copy(w.bitcast(jnp.uint32).at[:, pl.ds(col, width)], dst, ffn_sem.at[i])
        for i, (w, col, width, dst) in enumerate(ffn_pieces)]
    out_copies = [
        pltpu.make_async_copy(tile_ref.at[i],
                              outt_hbm.at[:, pl.ds(i * _LANES, _LANES)], tile_sem.at[i])
        for i in range(n_io)]

    def transpose_in(i):
        rows = pl.ds(pl.multiple_of(i * _LANES, _LANES), _LANES)
        res_ref[rows, :] = tile_ref[i].astype(jnp.float32).T

    def start(copies):
        for c in copies:
            c.start()

    n_first = pl.cdiv((_LAG + _EARLY) * seg, _LANES)
    per_group = pl.cdiv(n_io - n_first, n_groups)
    start([x_copy(i) for i in range(n_first)])
    start(head_copies(0))
    for i in range(n_first):
        x_copy(i).wait()
    for g in range(1, _COPIES_AHEAD):
        start(head_copies(g))
    start([x_copy(n_first + j) for j in range(per_group)])
    for i in range(n_first):
        transpose_in(i)
    early_h_ref[...] = _pack(normed(range(_LAG, _LAG + _EARLY)))

    @pl.loop(0, n_groups)
    def _load_group(g):
        pl.when(g + _COPIES_AHEAD < n_groups)(lambda: start(head_copies(g + _COPIES_AHEAD)))
        pl.when(g + _COPIES_AHEAD == n_groups)(lambda: start(wo_copies))
        pl.when(g == n_groups - _FFN_COPY_LEAD)(lambda: start(ffn_copies))
        tiles = [n_first + g * per_group + j for j in range(per_group)]
        for i in tiles:
            pl.when(i + per_group < n_io)(lambda i=i: x_copy(i + per_group).start())
            pl.when(i < n_io)(lambda i=i: x_copy(i).wait())
        for c in head_copies(g):
            c.wait()
        for p in range(pairs):
            for i in range(3):
                words = stage_ref[g, 3 * p + i]
                lo = pltpu.bitcast(words << 16, jnp.float32)
                hi = pltpu.bitcast(words & jnp.uint32(0xFFFF0000), jnp.float32)
                for head, w in enumerate((lo, hi)):
                    col = (3 * (2 * p + head) + i) * d_head
                    wqkv_ref[g, :, col:col + d_head] = _pack(w.astype(jnp.bfloat16))
        early_ref[g] = _pack(projector(_unpack(early_h_ref[...]))(g))
        for i in tiles:
            transpose_in(jnp.minimum(i, n_io - 1))

    for c in wo_copies:
        c.wait()

    mem0 = mem0_ref[...].astype(jnp.float32)
    mem1 = jax.lax.fori_loop(0, _LAG, single_step, mem0)
    for c in ffn_copies:
        c.wait()
    ffn_only(0)
    h_ref[:2 * n_mem, :] = jnp.concatenate([mem1, mem0], axis=0).astype(jnp.bfloat16)
    h_ref[2 * n_mem:, :] = normed([_LAG, n_seg])
    jax.lax.fori_loop(0, 2, functools.partial(double_step, early=True, with_ffn=False), mem0)
    jax.lax.fori_loop(2, _EARLY, functools.partial(double_step, early=True), mem0)
    mem2 = jax.lax.fori_loop(_EARLY, n_seg - _LAG, functools.partial(double_step, early=False),
                             mem0)

    n_done = (n_seg - _LAG - 8) * seg // _LANES + 1
    for i in range((_EARLY - 7) * seg // _LANES):
        transpose_out(i)
    start(out_copies[:n_done])
    last = 2 * n_seg - _LAG
    ffn_blocks = [n_seg - 2, n_seg - 1, last - 2, last - 1]
    mem2 = jax.lax.fori_loop(
        0, 2, lambda half, mem: single_step(last + half, mem, ffn_blocks, half), mem2)
    jax.lax.fori_loop(last + 2, 2 * n_seg, single_step, mem2)
    for i in range(n_done, n_io - 1):
        transpose_out(i)
        out_copies[i].start()
    ffn_only(last)
    transpose_out(n_io - 1)
    out_copies[n_io - 1].start()
    for c in out_copies:
        c.wait()


@functools.partial(jax.jit, static_argnames=("A_seg_len",))
def pallas_interleave_layers__memory_aug_recurrent_mem_tr__glu_gated_swiglu__prompt_kernel(
    A_x: jax.Array,
    A_mem0: jax.Array,
    A_Wq: jax.Array,
    A_Wk: jax.Array,
    A_Wv: jax.Array,
    A_Wo: jax.Array,
    A_seg_len: int,
    B_x: jax.Array,
    B_w1: jax.Array,
    B_w3: jax.Array,
    B_w2: jax.Array,
):
    del B_x
    _, n_tok, d_model = A_x.shape
    n_mem = A_mem0.shape[1]
    _, n_heads, d_head = A_Wq.shape
    d_ff = B_w1.shape[1]
    n_groups = n_heads // _HEADS_PER_GROUP
    group_cols = 3 * d_head * _HEADS_PER_GROUP
    early_words = _EARLY * A_seg_len // 2
    hbm = pl.BlockSpec(memory_space=pltpu.HBM)
    out_t = pl.pallas_call(
        functools.partial(_kernel, seg=A_seg_len),
        out_shape=jax.ShapeDtypeStruct((d_model, n_tok), A_x.dtype),
        in_specs=[hbm, pl.BlockSpec(memory_space=pltpu.VMEM)] + [hbm] * 7,
        out_specs=hbm,
        scratch_shapes=[
            pltpu.VMEM((n_tok // _LANES, d_model, _LANES), A_x.dtype),
            pltpu.VMEM((3 * n_tok, d_model), jnp.float32),
            pltpu.VMEM((2 * (n_mem + A_seg_len), d_model), jnp.bfloat16),
            pltpu.VMEM((early_words, d_model), jnp.uint32),
            pltpu.VMEM((n_groups, early_words, group_cols), jnp.uint32),
            pltpu.VMEM((n_groups, 3 * _HEADS_PER_GROUP // 2, d_model, d_head), jnp.uint32),
            pltpu.VMEM((n_groups, d_model // 2, group_cols), jnp.uint32),
            pltpu.VMEM((d_model // 2, n_heads * d_head), jnp.uint32),
            pltpu.VMEM((2, d_model // 2, d_ff), jnp.uint32),
            pltpu.VMEM((2, d_model // 2, d_ff // 2), jnp.uint32),
            pltpu.SemaphoreType.DMA((3 * n_heads // 2,)),
            pltpu.SemaphoreType.DMA((n_heads,)),
            pltpu.SemaphoreType.DMA((2 + 2 * d_ff // _FFN_CHUNK,)),
            pltpu.SemaphoreType.DMA((n_tok // _LANES,)),
        ],
        compiler_params=pltpu.CompilerParams(vmem_limit_bytes=110 * 1024 * 1024),
    )(A_x.reshape(n_tok, d_model).T, A_mem0.reshape(n_mem, d_model), A_Wq, A_Wk, A_Wv,
      A_Wo.transpose(0, 2, 1), B_w1, B_w3, B_w2.T)
    return out_t.T.reshape(A_x.shape)
```

```python
import functools
import math

import jax
import jax.numpy as jnp
import jax.experimental.pallas as pl
import jax.experimental.pallas.tpu as pltpu

_EPS = 1e-05
_MASKED = -1000000000.0
_LOG2E = math.log2(math.e)
_LANES = 128
_LAG = 4
_EARLY = 16
_HEADS_PER_GROUP = 4
_FFN_CHUNK = 256
_COPIES_AHEAD = 2
_FFN_COPY_LEAD = 2
_ORDER = (
    "P0 G0 P1 S0 G1 P2 S1 V0 G2 G3 P3 V1 G4 O0 S2 P4 V2 G5 O1 S3 P5 S4 V3 O2 G6 V4 G7 S5 "
    "P6 O3 S6 V5 P7 G8 O4 S7 V6 D0 O5 V7 O6 O7")
_ORDER_EARLY = (
    "P0 P1 G0 S0 G1 G2 G3 V0 P2 S1 P3 O0 G4 S2 V1 P4 V2 O1 G5 S3 P5 S4 V3 O2 V4 G6 G7 S5 "
    "P6 O3 S6 V5 P7 G8 O4 V6 S7 D0 O5 V7 O6 O7")
_ORDER_ATTENTION = (
    "P0 P1 S0 P2 S1 V0 P3 V1 O0 S2 P4 V2 O1 S3 P5 S4 V3 O2 S5 P6 O3 V4 S6 V5 P7 O4 S7 V6 "
    "O5 V7 O6 O7")


def _layernorm(x):
    m = jnp.mean(x, axis=-1, keepdims=True)
    d = x - m
    v = jnp.mean(d * d, axis=-1, keepdims=True)
    return d * jax.lax.rsqrt(v + _EPS)


def _dot(a, b):
    return jnp.dot(a, b, preferred_element_type=jnp.float32)


def _dot_nt(a, b):
    return jax.lax.dot_general(a, b, (((1,), (1,)), ((), ())),
                               preferred_element_type=jnp.float32)


def _pack(x):
    return pltpu.bitcast(x, jnp.uint32)


def _unpack(words):
    return pltpu.bitcast(words, jnp.bfloat16)


def _attention_masks(n_layers, n_mem, seg):
    rows = n_layers * (n_mem + seg)
    i = jax.lax.broadcasted_iota(jnp.int32, (rows, rows), 0)
    j = jax.lax.broadcasted_iota(jnp.int32, (rows, rows), 1)
    visible = (i < n_layers * n_mem) | (i >= j)
    if n_layers == 1:
        return visible, _MASKED * _LOG2E

    def second_layer(r):
        return ((r >= n_mem) & (r < 2 * n_mem)) | (r >= 2 * n_mem + seg)

    same = second_layer(i) == second_layer(j)
    fill = jnp.where(same, _MASKED * _LOG2E, -jnp.inf).astype(jnp.float32)
    return same & visible, fill


def _kernel(xt_hbm, mem0_ref, wq_hbm, wk_hbm, wv_hbm, wot_hbm, w1_hbm, w3_hbm, w2t_hbm,
            outt_hbm, tile_ref, res_ref, h_ref, early_h_ref, early_ref, stage_ref, wqkv_ref, wot_ref, w13_ref,
            w2t_ref, stage_sem, wo_sem, ffn_sem, tile_sem, *, seg):
    d_model, n_tok = xt_hbm.shape
    n_mem = mem0_ref.shape[0]
    _, n_heads, d_head = wq_hbm.shape
    n_groups = n_heads // _HEADS_PER_GROUP
    half_ff = w2t_ref.shape[2]
    n_chunks = half_ff // _FFN_CHUNK
    n_seg = n_tok // seg
    n_io = n_tok // _LANES
    score_scale = d_head ** -0.5 * _LOG2E

    def block(r):
        return pl.ds(pl.multiple_of(r * seg, seg), seg)

    def load_blocks(blocks):
        return jnp.concatenate([res_ref[block(r), :] for r in blocks], axis=0)

    def store_blocks(blocks, value):
        for i, r in enumerate(blocks):
            res_ref[block(r), :] = value[i * seg:(i + 1) * seg]

    def normed(blocks):
        return _layernorm(load_blocks(blocks)).astype(jnp.bfloat16)

    def transpose_out(i):
        rows = pl.ds(pl.multiple_of(2 * n_tok + i * _LANES, _LANES), _LANES)
        tile_ref[i] = res_ref[rows, :].T.astype(tile_ref.dtype)

    def gated(hn, half, c):
        cols = slice(2 * c * _FFN_CHUNK, 2 * (c + 1) * _FFN_CHUNK)
        both = _dot(hn, _unpack(w13_ref[half, :, cols]))
        gate, up = both[:, :_FFN_CHUNK], both[:, _FFN_CHUNK:]
        return (gate * jax.nn.sigmoid(gate) * up).astype(jnp.bfloat16)

    def mix(order, project, attn_blocks, ffn_blocks, half):
        n_layers = len(attn_blocks)
        visible, fill = _attention_masks(n_layers, n_mem, seg)
        if ffn_blocks:
            hn = normed(ffn_blocks)
        qkv, probs, heads, acts, out, y = {}, {}, {}, [], None, None

        def part(g, head, which):
            col = (3 * head + which) * d_head
            return qkv[g][:, col:col + d_head]

        for name in order.split():
            stage, g = name[0], int(name[1:])
            if stage in "GD" and not ffn_blocks:
                continue
            if stage == "P":
                qkv[g] = project(g)
            elif stage == "S":
                probs[g] = []
                for s in [_dot_nt(part(g, i, 0), part(g, i, 1)) for i in range(_HEADS_PER_GROUP)]:
                    s = jnp.where(visible, s * score_scale, fill)
                    p = jnp.exp2(s - jnp.max(s, axis=-1, keepdims=True))
                    inv = 1.0 / jnp.sum(p, axis=-1, keepdims=True)
                    probs[g].append((p.astype(jnp.bfloat16), inv))
            elif stage == "V":
                heads[g] = [(_dot(p, part(g, i, 2)) * inv).astype(jnp.bfloat16)
                            for i, (p, inv) in enumerate(probs[g])]
            elif stage == "O":
                width = _HEADS_PER_GROUP * d_head
                o = _dot_nt(jnp.concatenate(heads[g], axis=1),
                            _unpack(wot_ref[:, g * width:(g + 1) * width]))
                out = o if out is None else out + o
            elif stage == "G":
                acts.append(gated(hn, half, g))
            elif stage == "D":
                y = _dot_nt(_unpack(w2t_ref[half]), jnp.concatenate(acts, axis=1)).T
                y = y + load_blocks([r + half * n_seg for r in ffn_blocks])
        if ffn_blocks:
            store_blocks([r + n_seg for r in ffn_blocks], y)
        store_blocks(attn_blocks, load_blocks(attn_blocks) + out[n_layers * n_mem:])
        return out[:n_layers * n_mem], y

    def projector(h):
        return lambda g: _dot(h, _unpack(wqkv_ref[g])).astype(jnp.bfloat16)

    def single_step(r, mem, ffn_blocks=(), half=None):
        h = jnp.concatenate([mem, _layernorm(load_blocks([r]))], axis=0)
        order = _ORDER_EARLY if ffn_blocks else _ORDER_ATTENTION
        return mix(order, projector(h.astype(jnp.bfloat16)), [r], ffn_blocks, half)[0]

    def ffn_only(first):
        rows = pl.ds(first * seg, 4 * seg)
        y = res_ref[rows, :]
        hn = _layernorm(y).astype(jnp.bfloat16)
        for half in range(2):
            acts = jnp.concatenate([gated(hn, half, c) for c in range(n_chunks)], axis=1)
            y = y + _dot_nt(_unpack(w2t_ref[half]), acts).T
        res_ref[pl.ds((first + n_seg) * seg, 4 * seg), :] = y

    def double_step(b, _, *, early, with_ffn=True):
        half = b % 2
        f1, f2 = b - half + _LAG - 2, n_seg + b - half - 2
        if early:
            rest = projector(jnp.concatenate(
                [h_ref[:2 * n_mem, :], h_ref[2 * n_mem + seg:, :]], axis=0))
            rows = pl.ds(pl.multiple_of(b * (seg // 2), seg // 2), seg // 2)

            def project(g):
                qkv = rest(g)
                known = _unpack(early_ref[g, rows, :])
                return jnp.concatenate([qkv[:2 * n_mem], known, qkv[2 * n_mem:]], axis=0)
        else:
            project = projector(h_ref[...])
            transpose_out((b - 7) * seg // _LANES)
        h1 = normed([jnp.minimum(b + 1 + _LAG, n_seg - 1)])
        x2 = load_blocks([n_seg + b + 1 - half])
        order = (_ORDER_EARLY if early else _ORDER) if with_ffn else _ORDER_ATTENTION
        mems, y = mix(order, project, [b + _LAG, n_seg + b],
                      [f1, f1 + 1, f2, f2 + 1] if with_ffn else [], half)
        x2 = jnp.where(half == 1, y[:seg], x2) if with_ffn else load_blocks([n_seg + b + 1])
        h_ref[:2 * n_mem, :] = mems.astype(jnp.bfloat16)
        h_ref[2 * n_mem:2 * n_mem + seg, :] = h1
        h_ref[2 * n_mem + seg:, :] = _layernorm(x2).astype(jnp.bfloat16)
        return mems[n_mem:]

    pairs = _HEADS_PER_GROUP // 2

    def head_copies(g):
        return [pltpu.make_async_copy(w.bitcast(jnp.uint32).at[:, g * pairs + p, :],
                                      stage_ref.at[g, 3 * p + i], stage_sem.at[3 * (g * pairs + p) + i])
                for p in range(pairs) for i, w in enumerate((wq_hbm, wk_hbm, wv_hbm))]

    def x_copy(i):
        cols = pl.ds(pl.multiple_of(i * _LANES, _LANES), _LANES)
        return pltpu.make_async_copy(xt_hbm.at[:, cols], tile_ref.at[i], tile_sem.at[i])

    wo_copies = [
        pltpu.make_async_copy(wot_hbm.bitcast(jnp.uint32).at[h],
                              wot_ref.at[:, pl.ds(h * d_head, d_head)], wo_sem.at[h])
        for h in range(n_heads)]
    ffn_pieces = [(w2t_hbm, half * half_ff, half_ff, w2t_ref.at[half]) for half in range(2)]
    for half in range(2):
        for c in range(n_chunks):
            for i, w in enumerate((w1_hbm, w3_hbm)):
                dst = w13_ref.at[half, :, pl.ds((2 * c + i) * _FFN_CHUNK, _FFN_CHUNK)]
                ffn_pieces.append((w, half * half_ff + c * _FFN_CHUNK, _FFN_CHUNK, dst))
    ffn_copies = [
        pltpu.make_async_copy(w.bitcast(jnp.uint32).at[:, pl.ds(col, width)], dst, ffn_sem.at[i])
        for i, (w, col, width, dst) in enumerate(ffn_pieces)]
    out_copies = [
        pltpu.make_async_copy(tile_ref.at[i],
                              outt_hbm.at[:, pl.ds(i * _LANES, _LANES)], tile_sem.at[i])
        for i in range(n_io)]

    def transpose_in(i):
        rows = pl.ds(pl.multiple_of(i * _LANES, _LANES), _LANES)
        res_ref[rows, :] = tile_ref[i].astype(jnp.float32).T

    def start(copies):
        for c in copies:
            c.start()

    n_first = pl.cdiv((_LAG + _EARLY) * seg, _LANES)
    per_group = pl.cdiv(n_io - n_first, n_groups)
    start([x_copy(i) for i in range(n_first)])
    start(head_copies(0))
    for i in range(n_first):
        x_copy(i).wait()
    for g in range(1, _COPIES_AHEAD):
        start(head_copies(g))
    start([x_copy(n_first + j) for j in range(per_group)])
    for i in range(n_first):
        transpose_in(i)
    early_h_ref[...] = _pack(normed(range(_LAG, _LAG + _EARLY)))

    @pl.loop(0, n_groups)
    def _load_group(g):
        pl.when(g + _COPIES_AHEAD < n_groups)(lambda: start(head_copies(g + _COPIES_AHEAD)))
        pl.when(g + _COPIES_AHEAD == n_groups)(lambda: start(wo_copies))
        pl.when(g == n_groups - _FFN_COPY_LEAD)(lambda: start(ffn_copies))
        tiles = [n_first + g * per_group + j for j in range(per_group)]
        for i in tiles:
            pl.when(i + per_group < n_io)(lambda i=i: x_copy(i + per_group).start())
            pl.when(i < n_io)(lambda i=i: x_copy(i).wait())
        for c in head_copies(g):
            c.wait()
        for p in range(pairs):
            for i in range(3):
                words = stage_ref[g, 3 * p + i]
                lo = pltpu.bitcast(words << 16, jnp.float32)
                hi = pltpu.bitcast(words & jnp.uint32(0xFFFF0000), jnp.float32)
                for head, w in enumerate((lo, hi)):
                    col = (3 * (2 * p + head) + i) * d_head
                    wqkv_ref[g, :, col:col + d_head] = _pack(w.astype(jnp.bfloat16))
        early_ref[g] = _pack(projector(_unpack(early_h_ref[...]))(g))
        for i in tiles:
            transpose_in(jnp.minimum(i, n_io - 1))

    for c in wo_copies:
        c.wait()

    mem0 = mem0_ref[...].astype(jnp.float32)
    mem1 = jax.lax.fori_loop(0, _LAG, single_step, mem0)
    for c in ffn_copies:
        c.wait()
    ffn_only(0)
    h_ref[:2 * n_mem, :] = jnp.concatenate([mem1, mem0], axis=0).astype(jnp.bfloat16)
    h_ref[2 * n_mem:, :] = normed([_LAG, n_seg])
    jax.lax.fori_loop(0, 2, functools.partial(double_step, early=True, with_ffn=False), mem0)
    jax.lax.fori_loop(2, _EARLY, functools.partial(double_step, early=True), mem0)
    mem2 = jax.lax.fori_loop(_EARLY, n_seg - _LAG, functools.partial(double_step, early=False),
                             mem0)

    n_done = (n_seg - _LAG - 8) * seg // _LANES + 1
    for i in range((_EARLY - 7) * seg // _LANES):
        transpose_out(i)
    start(out_copies[:n_done])
    last = 2 * n_seg - _LAG
    ffn_blocks = [n_seg - 2, n_seg - 1, last - 2, last - 1]
    mem2 = jax.lax.fori_loop(
        0, 2, lambda half, mem: single_step(last + half, mem, ffn_blocks, half), mem2)
    jax.lax.fori_loop(last + 2, 2 * n_seg, single_step, mem2)
    for i in range(n_done, n_io - 1):
        transpose_out(i)
        out_copies[i].start()
    ffn_only(last)
    transpose_out(n_io - 1)
    out_copies[n_io - 1].start()
    for c in out_copies:
        c.wait()


@functools.partial(jax.jit, static_argnames=("A_seg_len",))
def pallas_interleave_layers__memory_aug_recurrent_mem_tr__glu_gated_swiglu__prompt_kernel(
    A_x: jax.Array,
    A_mem0: jax.Array,
    A_Wq: jax.Array,
    A_Wk: jax.Array,
    A_Wv: jax.Array,
    A_Wo: jax.Array,
    A_seg_len: int,
    B_x: jax.Array,
    B_w1: jax.Array,
    B_w3: jax.Array,
    B_w2: jax.Array,
):
    del B_x
    _, n_tok, d_model = A_x.shape
    n_mem = A_mem0.shape[1]
    _, n_heads, d_head = A_Wq.shape
    d_ff = B_w1.shape[1]
    n_groups = n_heads // _HEADS_PER_GROUP
    group_cols = 3 * d_head * _HEADS_PER_GROUP
    early_words = _EARLY * A_seg_len // 2
    hbm = pl.BlockSpec(memory_space=pltpu.HBM)
    out_t = pl.pallas_call(
        functools.partial(_kernel, seg=A_seg_len),
        out_shape=jax.ShapeDtypeStruct((d_model, n_tok), A_x.dtype),
        in_specs=[hbm, pl.BlockSpec(memory_space=pltpu.VMEM)] + [hbm] * 7,
        out_specs=hbm,
        scratch_shapes=[
            pltpu.VMEM((n_tok // _LANES, d_model, _LANES), A_x.dtype),
            pltpu.VMEM((3 * n_tok, d_model), jnp.float32),
            pltpu.VMEM((2 * (n_mem + A_seg_len), d_model), jnp.bfloat16),
            pltpu.VMEM((early_words, d_model), jnp.uint32),
            pltpu.VMEM((n_groups, early_words, group_cols), jnp.uint32),
            pltpu.VMEM((n_groups, 3 * _HEADS_PER_GROUP // 2, d_model, d_head), jnp.uint32),
            pltpu.VMEM((n_groups, d_model // 2, group_cols), jnp.uint32),
            pltpu.VMEM((d_model // 2, n_heads * d_head), jnp.uint32),
            pltpu.VMEM((2, d_model // 2, d_ff), jnp.uint32),
            pltpu.VMEM((2, d_model // 2, d_ff // 2), jnp.uint32),
            pltpu.SemaphoreType.DMA((3 * n_heads // 2,)),
            pltpu.SemaphoreType.DMA((n_heads,)),
            pltpu.SemaphoreType.DMA((2 + 2 * d_ff // _FFN_CHUNK,)),
            pltpu.SemaphoreType.DMA((n_tok // _LANES,)),
        ],
        compiler_params=pltpu.CompilerParams(vmem_limit_bytes=110 * 1024 * 1024),
    )(A_x.reshape(n_tok, d_model).T, A_mem0.reshape(n_mem, d_model), A_Wq, A_Wk, A_Wv,
      A_Wo.transpose(0, 2, 1), B_w1, B_w3, B_w2.T)
    return out_t.T.reshape(A_x.shape)
```

```python
import functools
import math

import jax
import jax.numpy as jnp
import jax.experimental.pallas as pl
import jax.experimental.pallas.tpu as pltpu

_EPS = 1e-05
_MASKED = -1000000000.0
_LOG2E = math.log2(math.e)
_LANES = 128
_LAG = 4
_EARLY = 16
_HEADS_PER_GROUP = 4
_FFN_CHUNK = 256
_COPIES_AHEAD = 2
_WO_COPY_LEAD = 2
_FFN_COPY_LEAD = 2
_ORDER = (
    "P0 G0 P1 S0 G1 P2 S1 V0 G2 G3 P3 V1 G4 O0 S2 P4 V2 G5 O1 S3 P5 S4 V3 O2 G6 V4 G7 S5 "
    "P6 O3 S6 V5 P7 G8 O4 S7 V6 D0 O5 V7 O6 O7")
_ORDER_EARLY = (
    "P0 P1 G0 S0 G1 G2 G3 V0 P2 S1 P3 O0 G4 S2 V1 P4 V2 O1 G5 S3 P5 S4 V3 O2 V4 G6 G7 S5 "
    "P6 O3 S6 V5 P7 G8 O4 V6 S7 D0 O5 V7 O6 O7")
_ORDER_ATTENTION = (
    "P0 P1 S0 P2 S1 V0 P3 V1 O0 S2 P4 V2 O1 S3 P5 S4 V3 O2 S5 P6 O3 V4 S6 V5 P7 O4 S7 V6 "
    "O5 V7 O6 O7")


def _layernorm(x):
    m = jnp.mean(x, axis=-1, keepdims=True)
    d = x - m
    v = jnp.mean(d * d, axis=-1, keepdims=True)
    return d * jax.lax.rsqrt(v + _EPS)


def _dot(a, b):
    return jnp.dot(a, b, preferred_element_type=jnp.float32)


def _dot_nt(a, b):
    return jax.lax.dot_general(a, b, (((1,), (1,)), ((), ())),
                               preferred_element_type=jnp.float32)


def _pack(x):
    return pltpu.bitcast(x, jnp.uint32)


def _unpack(words):
    return pltpu.bitcast(words, jnp.bfloat16)


def _attention_masks(n_layers, n_mem, seg):
    rows = n_layers * (n_mem + seg)
    i = jax.lax.broadcasted_iota(jnp.int32, (rows, rows), 0)
    j = jax.lax.broadcasted_iota(jnp.int32, (rows, rows), 1)
    visible = (i < n_layers * n_mem) | (i >= j)
    if n_layers == 1:
        return visible, _MASKED * _LOG2E

    def second_layer(r):
        return ((r >= n_mem) & (r < 2 * n_mem)) | (r >= 2 * n_mem + seg)

    same = second_layer(i) == second_layer(j)
    fill = jnp.where(same, _MASKED * _LOG2E, -jnp.inf).astype(jnp.float32)
    return same & visible, fill


def _kernel(xt_hbm, mem0_ref, wq_hbm, wk_hbm, wv_hbm, wot_hbm, w1_hbm, w3_hbm, w2t_hbm,
            outt_hbm, tile_ref, res_ref, h_ref, early_h_ref, early_ref, stage_ref, wqkv_ref, wot_ref,
            w1_ref, w3_ref, w2t_ref, stage_sem, weight_sem, tile_sem, *, seg):
    d_model, n_tok = xt_hbm.shape
    n_mem = mem0_ref.shape[0]
    _, n_heads, d_head = wq_hbm.shape
    n_groups = n_heads // _HEADS_PER_GROUP
    half_ff = w2t_ref.shape[2]
    n_chunks = half_ff // _FFN_CHUNK
    n_seg = n_tok // seg
    n_io = n_tok // _LANES
    score_scale = d_head ** -0.5 * _LOG2E

    def block(r):
        return pl.ds(pl.multiple_of(r * seg, seg), seg)

    def load_blocks(blocks):
        return jnp.concatenate([res_ref[block(r), :] for r in blocks], axis=0)

    def store_blocks(blocks, value):
        for i, r in enumerate(blocks):
            res_ref[block(r), :] = value[i * seg:(i + 1) * seg]

    def normed(blocks):
        return _layernorm(load_blocks(blocks)).astype(jnp.bfloat16)

    def transpose_out(i):
        rows = pl.ds(pl.multiple_of(2 * n_tok + i * _LANES, _LANES), _LANES)
        tile_ref[i] = res_ref[rows, :].T.astype(tile_ref.dtype)

    def gated(hn, half, c):
        cols = slice(c * _FFN_CHUNK, (c + 1) * _FFN_CHUNK)
        both = _dot(hn, _unpack(
            jnp.concatenate([w1_ref[half, :, cols], w3_ref[half, :, cols]], axis=1)))
        gate, up = both[:, :_FFN_CHUNK], both[:, _FFN_CHUNK:]
        return (gate * jax.nn.sigmoid(gate) * up).astype(jnp.bfloat16)

    def mix(order, project, attn_blocks, ffn_blocks, half):
        n_layers = len(attn_blocks)
        visible, fill = _attention_masks(n_layers, n_mem, seg)
        if ffn_blocks:
            hn = normed(ffn_blocks)
        qkv, probs, heads, acts, out, y = {}, {}, {}, [], None, None

        def part(g, head, which):
            col = (3 * head + which) * d_head
            return qkv[g][:, col:col + d_head]

        for name in order.split():
            stage, g = name[0], int(name[1:])
            if stage in "GD" and not ffn_blocks:
                continue
            if stage == "P":
                qkv[g] = project(g)
            elif stage == "S":
                probs[g] = []
                for s in [_dot_nt(part(g, i, 0), part(g, i, 1)) for i in range(_HEADS_PER_GROUP)]:
                    s = jnp.where(visible, s * score_scale, fill)
                    p = jnp.exp2(s - jnp.max(s, axis=-1, keepdims=True))
                    inv = 1.0 / jnp.sum(p, axis=-1, keepdims=True)
                    probs[g].append((p.astype(jnp.bfloat16), inv))
            elif stage == "V":
                heads[g] = [(_dot(p, part(g, i, 2)) * inv).astype(jnp.bfloat16)
                            for i, (p, inv) in enumerate(probs[g])]
            elif stage == "O":
                wo = [wot_ref[g * _HEADS_PER_GROUP + i] for i in range(_HEADS_PER_GROUP)]
                o = _dot_nt(jnp.concatenate(heads[g], axis=1),
                            _unpack(jnp.concatenate(wo, axis=1)))
                out = o if out is None else out + o
            elif stage == "G":
                acts.append(gated(hn, half, g))
            elif stage == "D":
                y = _dot_nt(_unpack(w2t_ref[half]), jnp.concatenate(acts, axis=1)).T
                y = y + load_blocks([r + half * n_seg for r in ffn_blocks])
        if ffn_blocks:
            store_blocks([r + n_seg for r in ffn_blocks], y)
        store_blocks(attn_blocks, load_blocks(attn_blocks) + out[n_layers * n_mem:])
        return out[:n_layers * n_mem], y

    def projector(h):
        return lambda g: _dot(h, _unpack(wqkv_ref[g])).astype(jnp.bfloat16)

    def single_step(r, mem, ffn_blocks=(), half=None):
        h = jnp.concatenate([mem, _layernorm(load_blocks([r]))], axis=0)
        order = _ORDER_EARLY if ffn_blocks else _ORDER_ATTENTION
        return mix(order, projector(h.astype(jnp.bfloat16)), [r], ffn_blocks, half)[0]

    def ffn_only(first):
        rows = pl.ds(first * seg, 4 * seg)
        y = res_ref[rows, :]
        hn = _layernorm(y).astype(jnp.bfloat16)
        for half in range(2):
            acts = jnp.concatenate([gated(hn, half, c) for c in range(n_chunks)], axis=1)
            y = y + _dot_nt(_unpack(w2t_ref[half]), acts).T
        res_ref[pl.ds((first + n_seg) * seg, 4 * seg), :] = y

    def double_step(b, _, *, early, with_ffn=True):
        half = b % 2
        f1, f2 = b - half + _LAG - 2, n_seg + b - half - 2
        if early:
            rest = projector(jnp.concatenate(
                [h_ref[:2 * n_mem, :], h_ref[2 * n_mem + seg:, :]], axis=0))
            rows = pl.ds(pl.multiple_of(b * (seg // 2), seg // 2), seg // 2)

            def project(g):
                qkv = rest(g)
                known = _unpack(early_ref[g, rows, :])
                return jnp.concatenate([qkv[:2 * n_mem], known, qkv[2 * n_mem:]], axis=0)
        else:
            project = projector(h_ref[...])
            transpose_out((b - 7) * seg // _LANES)
        h1 = normed([jnp.minimum(b + 1 + _LAG, n_seg - 1)])
        x2 = load_blocks([n_seg + b + 1 - half])
        order = _ORDER_EARLY if early and with_ffn else _ORDER
        mems, y = mix(order, project, [b + _LAG, n_seg + b],
                      [f1, f1 + 1, f2, f2 + 1] if with_ffn else [], half)
        x2 = jnp.where(half == 1, y[:seg], x2) if with_ffn else load_blocks([n_seg + b + 1])
        h_ref[:2 * n_mem, :] = mems.astype(jnp.bfloat16)
        h_ref[2 * n_mem:2 * n_mem + seg, :] = h1
        h_ref[2 * n_mem + seg:, :] = _layernorm(x2).astype(jnp.bfloat16)
        return mems[n_mem:]

    pairs = _HEADS_PER_GROUP // 2

    def head_copies(g):
        return [pltpu.make_async_copy(w.bitcast(jnp.uint32).at[:, g * pairs + p, :],
                                      stage_ref.at[g, 3 * p + i], stage_sem.at[3 * (g * pairs + p) + i])
                for p in range(pairs) for i, w in enumerate((wq_hbm, wk_hbm, wv_hbm))]

    def x_copy(i):
        cols = pl.ds(pl.multiple_of(i * _LANES, _LANES), _LANES)
        return pltpu.make_async_copy(xt_hbm.at[:, cols], tile_ref.at[i], tile_sem.at[i])

    wo_copies = [pltpu.make_async_copy(wot_hbm.bitcast(jnp.uint32), wot_ref, weight_sem.at[0])]
    ffn_copies = [
        pltpu.make_async_copy(src.bitcast(jnp.uint32).at[:, pl.ds(half * half_ff, half_ff)],
                              dst.at[half], weight_sem.at[1 + 2 * i + half])
        for half in range(2)
        for i, (src, dst) in enumerate(((w1_hbm, w1_ref), (w3_hbm, w3_ref), (w2t_hbm, w2t_ref)))]

    out_copies = [
        pltpu.make_async_copy(tile_ref.at[i],
                              outt_hbm.at[:, pl.ds(i * _LANES, _LANES)], tile_sem.at[i])
        for i in range(n_io)]

    def transpose_in(i):
        rows = pl.ds(pl.multiple_of(i * _LANES, _LANES), _LANES)
        res_ref[rows, :] = tile_ref[i].astype(jnp.float32).T

    def start(copies):
        for c in copies:
            c.start()

    n_first = pl.cdiv((_LAG + _EARLY) * seg, _LANES)
    per_group = pl.cdiv(n_io - n_first, n_groups)
    start([x_copy(i) for i in range(n_first)])
    start(head_copies(0))
    for i in range(n_first):
        x_copy(i).wait()
    for g in range(1, _COPIES_AHEAD):
        start(head_copies(g))
    start([x_copy(n_first + j) for j in range(per_group)])
    for i in range(n_first):
        transpose_in(i)
    early_h_ref[...] = _pack(normed(range(_LAG, _LAG + _EARLY)))

    def split_heads(g, c):
        tiles = []
        for t in range(c * _HEADS_PER_GROUP, (c + 1) * _HEADS_PER_GROUP):
            head, which = divmod(t, 3)
            words = stage_ref[g, 3 * (head // 2) + which]
            words = words & jnp.uint32(0xFFFF0000) if head % 2 else words << 16
            tiles.append(pltpu.bitcast(words, jnp.float32).astype(jnp.bfloat16))
        return jnp.concatenate(tiles, axis=1)

    @pl.loop(0, n_groups)
    def _load_group(g):
        tiles = [n_first + g * per_group + j for j in range(per_group)]
        for i in tiles:
            pl.when(i + per_group < n_io)(lambda i=i: x_copy(i + per_group).start())
        pl.when(g + _COPIES_AHEAD < n_groups)(lambda: start(head_copies(g + _COPIES_AHEAD)))
        pl.when(g == n_groups - _WO_COPY_LEAD)(lambda: start(wo_copies))
        pl.when(g == n_groups - _FFN_COPY_LEAD)(lambda: start(ffn_copies))
        for i in tiles:
            pl.when(i < n_io)(lambda i=i: x_copy(i).wait())
        for c in head_copies(g):
            c.wait()
        h = _unpack(early_h_ref[...])
        width = _HEADS_PER_GROUP * d_head
        weights = split_heads(g, 0)
        for c in range(3):
            following = split_heads(g, c + 1) if c < 2 else None
            cols = slice(c * width, (c + 1) * width)
            wqkv_ref[g, :, cols] = _pack(weights)
            early_ref[g, :, cols] = _pack(_dot(h, weights).astype(jnp.bfloat16))
            weights = following
        for i in tiles:
            transpose_in(jnp.minimum(i, n_io - 1))

    for c in wo_copies:
        c.wait()

    mem0 = mem0_ref[...].astype(jnp.float32)
    mem1 = jax.lax.fori_loop(0, _LAG, single_step, mem0)
    for c in ffn_copies:
        c.wait()
    ffn_only(0)
    h_ref[:2 * n_mem, :] = jnp.concatenate([mem1, mem0], axis=0).astype(jnp.bfloat16)
    h_ref[2 * n_mem:, :] = normed([_LAG, n_seg])
    jax.lax.fori_loop(0, 2, functools.partial(double_step, early=True, with_ffn=False), mem0)
    jax.lax.fori_loop(2, _EARLY, functools.partial(double_step, early=True), mem0)
    mem2 = jax.lax.fori_loop(_EARLY, n_seg - _LAG, functools.partial(double_step, early=False),
                             mem0)

    n_done = (n_seg - _LAG - 8) * seg // _LANES + 1
    for i in range((_EARLY - 7) * seg // _LANES):
        transpose_out(i)
    start(out_copies[:n_done])
    last = 2 * n_seg - _LAG
    ffn_blocks = [n_seg - 2, n_seg - 1, last - 2, last - 1]
    mem2 = jax.lax.fori_loop(
        0, 2, lambda half, mem: single_step(last + half, mem, ffn_blocks, half), mem2)
    jax.lax.fori_loop(last + 2, 2 * n_seg, single_step, mem2)
    for i in range(n_done, n_io - 1):
        transpose_out(i)
        out_copies[i].start()
    ffn_only(last)
    transpose_out(n_io - 1)
    out_copies[n_io - 1].start()
    for c in out_copies:
        c.wait()


@functools.partial(jax.jit, static_argnames=("A_seg_len",))
def pallas_interleave_layers__memory_aug_recurrent_mem_tr__glu_gated_swiglu__prompt_kernel(
    A_x: jax.Array,
    A_mem0: jax.Array,
    A_Wq: jax.Array,
    A_Wk: jax.Array,
    A_Wv: jax.Array,
    A_Wo: jax.Array,
    A_seg_len: int,
    B_x: jax.Array,
    B_w1: jax.Array,
    B_w3: jax.Array,
    B_w2: jax.Array,
):
    del B_x
    _, n_tok, d_model = A_x.shape
    n_mem = A_mem0.shape[1]
    _, n_heads, d_head = A_Wq.shape
    d_ff = B_w1.shape[1]
    n_groups = n_heads // _HEADS_PER_GROUP
    group_cols = 3 * d_head * _HEADS_PER_GROUP
    early_words = _EARLY * A_seg_len // 2
    hbm = pl.BlockSpec(memory_space=pltpu.HBM)
    out_t = pl.pallas_call(
        functools.partial(_kernel, seg=A_seg_len),
        out_shape=jax.ShapeDtypeStruct((d_model, n_tok), A_x.dtype),
        in_specs=[hbm, pl.BlockSpec(memory_space=pltpu.VMEM)] + [hbm] * 7,
        out_specs=hbm,
        scratch_shapes=[
            pltpu.VMEM((n_tok // _LANES, d_model, _LANES), A_x.dtype),
            pltpu.VMEM((3 * n_tok, d_model), jnp.float32),
            pltpu.VMEM((2 * (n_mem + A_seg_len), d_model), jnp.bfloat16),
            pltpu.VMEM((early_words, d_model), jnp.uint32),
            pltpu.VMEM((n_groups, early_words, group_cols), jnp.uint32),
            pltpu.VMEM((n_groups, 3 * _HEADS_PER_GROUP // 2, d_model, d_head), jnp.uint32),
            pltpu.VMEM((n_groups, d_model // 2, group_cols), jnp.uint32),
            pltpu.VMEM((n_heads, d_model // 2, d_head), jnp.uint32),
            pltpu.VMEM((2, d_model // 2, d_ff // 2), jnp.uint32),
            pltpu.VMEM((2, d_model // 2, d_ff // 2), jnp.uint32),
            pltpu.VMEM((2, d_model // 2, d_ff // 2), jnp.uint32),
            pltpu.SemaphoreType.DMA((3 * n_heads // 2,)),
            pltpu.SemaphoreType.DMA((7,)),
            pltpu.SemaphoreType.DMA((n_tok // _LANES,)),
        ],
        compiler_params=pltpu.CompilerParams(vmem_limit_bytes=110 * 1024 * 1024),
    )(A_x.reshape(n_tok, d_model).T, A_mem0.reshape(n_mem, d_model), A_Wq, A_Wk, A_Wv,
      A_Wo.transpose(0, 2, 1), B_w1, B_w3, B_w2.T)
    return out_t.T.reshape(A_x.shape)
```

```python
import functools
import math

import jax
import jax.numpy as jnp
import jax.experimental.pallas as pl
import jax.experimental.pallas.tpu as pltpu

_EPS = 1e-05
_MASKED = -1000000000.0
_LOG2E = math.log2(math.e)
_LANES = 128
_LAG = 4
_EARLY = 16
_HEADS_PER_GROUP = 4
_FFN_CHUNK = 256
_COPIES_AHEAD = 2
_WO_COPY_LEAD = 2
_FFN_COPY_LEAD = 2
_ORDER = (
    "P0 G0 P1 S0 G1 P2 S1 V0 G2 G3 P3 V1 G4 O0 S2 P4 V2 G5 O1 S3 P5 S4 V3 O2 G6 V4 G7 S5 "
    "P6 O3 S6 V5 P7 G8 O4 S7 V6 D0 O5 V7 O6 O7")
_ORDER_EARLY = (
    "P0 P1 G0 S0 G1 G2 G3 V0 P2 S1 P3 O0 G4 S2 V1 P4 V2 O1 G5 S3 P5 S4 V3 O2 V4 G6 G7 S5 "
    "P6 O3 S6 V5 P7 G8 O4 V6 S7 D0 O5 V7 O6 O7")
_ORDER_ATTENTION = (
    "P0 P1 S0 P2 S1 V0 P3 V1 O0 S2 P4 V2 O1 S3 P5 S4 V3 O2 S5 P6 O3 V4 S6 V5 P7 O4 S7 V6 "
    "O5 V7 O6 O7")


def _layernorm(x):
    m = jnp.mean(x, axis=-1, keepdims=True)
    d = x - m
    v = jnp.mean(d * d, axis=-1, keepdims=True)
    return d * jax.lax.rsqrt(v + _EPS)


def _dot(a, b):
    return jnp.dot(a, b, preferred_element_type=jnp.float32)


def _dot_nt(a, b):
    return jax.lax.dot_general(a, b, (((1,), (1,)), ((), ())),
                               preferred_element_type=jnp.float32)


def _pack(x):
    return pltpu.bitcast(x, jnp.uint32)


def _unpack(words):
    return pltpu.bitcast(words, jnp.bfloat16)


def _attention_masks(n_layers, n_mem, seg):
    rows = n_layers * (n_mem + seg)
    i = jax.lax.broadcasted_iota(jnp.int32, (rows, rows), 0)
    j = jax.lax.broadcasted_iota(jnp.int32, (rows, rows), 1)
    visible = (i < n_layers * n_mem) | (i >= j)
    if n_layers == 1:
        return visible, _MASKED * _LOG2E

    def second_layer(r):
        return ((r >= n_mem) & (r < 2 * n_mem)) | (r >= 2 * n_mem + seg)

    same = second_layer(i) == second_layer(j)
    fill = jnp.where(same, _MASKED * _LOG2E, -jnp.inf).astype(jnp.float32)
    return same & visible, fill


def _kernel(xt_hbm, mem0_hbm, wq_hbm, wk_hbm, wv_hbm, wot_hbm, w1_hbm, w3_hbm, w2t_hbm,
            outt_hbm, mem0_ref, tile_ref, res_ref, h_ref, early_h_ref, early_ref, spare_ref,
            stage_ref, wqkv_ref, wot_ref,
            w1_ref, w3_ref, w2t_ref, stage_sem, weight_sem, tile_sem, *, seg):
    d_model, n_tok = xt_hbm.shape
    n_mem = mem0_ref.shape[0]
    _, n_heads, d_head = wq_hbm.shape
    n_groups = n_heads // _HEADS_PER_GROUP
    half_ff = w2t_ref.shape[2]
    n_chunks = half_ff // _FFN_CHUNK
    n_seg = n_tok // seg
    n_io = n_tok // _LANES
    score_scale = d_head ** -0.5 * _LOG2E

    def block(r):
        return pl.ds(pl.multiple_of(r * seg, seg), seg)

    def load_blocks(blocks):
        return jnp.concatenate([res_ref[block(r), :] for r in blocks], axis=0)

    def store_blocks(blocks, value):
        for i, r in enumerate(blocks):
            res_ref[block(r), :] = value[i * seg:(i + 1) * seg]

    def normed(blocks):
        return _layernorm(load_blocks(blocks)).astype(jnp.bfloat16)

    def transpose_out(i):
        rows = pl.ds(pl.multiple_of(2 * n_tok + i * _LANES, _LANES), _LANES)
        tile_ref[i] = res_ref[rows, :].T.astype(tile_ref.dtype)

    def gated(hn, half, c):
        cols = slice(c * _FFN_CHUNK, (c + 1) * _FFN_CHUNK)
        both = _dot(hn, _unpack(
            jnp.concatenate([w1_ref[half, :, cols], w3_ref[half, :, cols]], axis=1)))
        gate, up = both[:, :_FFN_CHUNK], both[:, _FFN_CHUNK:]
        return (gate * jax.nn.sigmoid(gate) * up).astype(jnp.bfloat16)

    def mix(order, project, attn_blocks, ffn_blocks, half):
        n_layers = len(attn_blocks)
        visible, fill = _attention_masks(n_layers, n_mem, seg)
        if ffn_blocks:
            hn = normed(ffn_blocks)
        qkv, probs, heads, acts, out, y = {}, {}, {}, [], None, None

        def part(g, head, which):
            col = (3 * head + which) * d_head
            return qkv[g][:, col:col + d_head]

        for name in order.split():
            stage, g = name[0], int(name[1:])
            if stage in "GD" and not ffn_blocks:
                continue
            if stage == "P":
                qkv[g] = project(g)
            elif stage == "S":
                probs[g] = []
                for s in [_dot_nt(part(g, i, 0), part(g, i, 1)) for i in range(_HEADS_PER_GROUP)]:
                    s = jnp.where(visible, s * score_scale, fill)
                    p = jnp.exp2(s - jnp.max(s, axis=-1, keepdims=True))
                    inv = 1.0 / jnp.sum(p, axis=-1, keepdims=True)
                    probs[g].append((p.astype(jnp.bfloat16), inv))
            elif stage == "V":
                heads[g] = [(_dot(p, part(g, i, 2)) * inv).astype(jnp.bfloat16)
                            for i, (p, inv) in enumerate(probs[g])]
            elif stage == "O":
                wo = [wot_ref[g * _HEADS_PER_GROUP + i] for i in range(_HEADS_PER_GROUP)]
                o = _dot_nt(jnp.concatenate(heads[g], axis=1),
                            _unpack(jnp.concatenate(wo, axis=1)))
                out = o if out is None else out + o
            elif stage == "G":
                acts.append(gated(hn, half, g))
            elif stage == "D":
                y = _dot_nt(_unpack(w2t_ref[half]), jnp.concatenate(acts, axis=1)).T
                y = y + load_blocks([r + half * n_seg for r in ffn_blocks])
        if ffn_blocks:
            store_blocks([r + n_seg for r in ffn_blocks], y)
        store_blocks(attn_blocks, load_blocks(attn_blocks) + out[n_layers * n_mem:])
        return out[:n_layers * n_mem], y

    def projector(h):
        return lambda g: _dot(h, _unpack(wqkv_ref[g])).astype(jnp.bfloat16)

    def single_step(r, mem, ffn_blocks=(), half=None):
        h = jnp.concatenate([mem, _layernorm(load_blocks([r]))], axis=0)
        order = _ORDER_EARLY if ffn_blocks else _ORDER_ATTENTION
        return mix(order, projector(h.astype(jnp.bfloat16)), [r], ffn_blocks, half)[0]

    def first_step(r, mem):
        spare = seg // _LAG
        rows = pl.ds(pl.multiple_of(r * spare, spare), spare)
        ahead = res_ref[pl.ds(pl.multiple_of((_LAG + _EARLY) * seg + r * spare, spare), spare), :]
        x = jnp.concatenate([load_blocks([r]), ahead], axis=0)
        h = jnp.concatenate([mem, _layernorm(x)], axis=0).astype(jnp.bfloat16)

        def project(g):
            qkv = _dot(h, _unpack(wqkv_ref[g]))
            spare_ref[g, rows, :] = qkv[n_mem + seg:]
            return qkv[:n_mem + seg].astype(jnp.bfloat16)

        return mix(_ORDER_ATTENTION, project, [r], (), None)[0]

    def ffn_transposed(first):
        x = res_ref[first * seg:(first + 4) * seg, :]
        hn = _layernorm(x).astype(jnp.bfloat16)
        halves = [
            _dot_nt(_unpack(w2t_ref[half]),
                    jnp.concatenate([gated(hn, half, c) for c in range(n_chunks)], axis=1))
            for half in range(2)]
        return halves[0] + halves[1], x

    def double_step(b, _, *, early, with_ffn=True):
        half = b % 2
        f1, f2 = b - half + _LAG - 2, n_seg + b - half - 2
        if early:
            rest = projector(jnp.concatenate(
                [h_ref[:2 * n_mem, :], h_ref[2 * n_mem + seg:, :]], axis=0))
            rows = pl.ds(pl.multiple_of(b * (seg // 2), seg // 2), seg // 2)

            def project(g):
                qkv = rest(g)
                known = _unpack(early_ref[g, rows, :])
                return jnp.concatenate([qkv[:2 * n_mem], known, qkv[2 * n_mem:]], axis=0)
        else:
            project = projector(h_ref[...])
            transpose_out((b - 7) * seg // _LANES)
        h1 = normed([jnp.minimum(b + 1 + _LAG, n_seg - 1)])
        x2 = load_blocks([n_seg + b + 1 - half])
        order = _ORDER_EARLY if early and with_ffn else _ORDER
        mems, y = mix(order, project, [b + _LAG, n_seg + b],
                      [f1, f1 + 1, f2, f2 + 1] if with_ffn else [], half)
        x2 = jnp.where(half == 1, y[:seg], x2) if with_ffn else load_blocks([n_seg + b + 1])
        h_ref[:2 * n_mem, :] = mems.astype(jnp.bfloat16)
        h_ref[2 * n_mem:2 * n_mem + seg, :] = h1
        h_ref[2 * n_mem + seg:, :] = _layernorm(x2).astype(jnp.bfloat16)
        return mems[n_mem:]

    pairs = _HEADS_PER_GROUP // 2

    def head_copies(g):
        return [pltpu.make_async_copy(w.bitcast(jnp.uint32).at[:, g * pairs + p, :],
                                      stage_ref.at[g, 3 * p + i], stage_sem.at[3 * (g * pairs + p) + i])
                for p in range(pairs) for i, w in enumerate((wq_hbm, wk_hbm, wv_hbm))]

    def x_copy(i):
        cols = pl.ds(pl.multiple_of(i * _LANES, _LANES), _LANES)
        return pltpu.make_async_copy(xt_hbm.at[:, cols], tile_ref.at[i], tile_sem.at[i])

    wo_copies = [pltpu.make_async_copy(wot_hbm.bitcast(jnp.uint32), wot_ref, weight_sem.at[0]),
                 pltpu.make_async_copy(mem0_hbm, mem0_ref, weight_sem.at[7])]
    ffn_copies = [
        pltpu.make_async_copy(src.bitcast(jnp.uint32).at[:, pl.ds(half * half_ff, half_ff)],
                              dst.at[half], weight_sem.at[1 + 2 * i + half])
        for half in range(2)
        for i, (src, dst) in enumerate(((w1_hbm, w1_ref), (w3_hbm, w3_ref), (w2t_hbm, w2t_ref)))]

    out_copies = [
        pltpu.make_async_copy(tile_ref.at[i],
                              outt_hbm.at[:, pl.ds(i * _LANES, _LANES)], tile_sem.at[i])
        for i in range(n_io)]

    def transpose_in(i):
        rows = pl.ds(pl.multiple_of(i * _LANES, _LANES), _LANES)
        res_ref[rows, :] = tile_ref[i].astype(jnp.float32).T

    def start(copies):
        for c in copies:
            c.start()

    n_first = pl.cdiv((_LAG + _EARLY) * seg, _LANES)
    per_group = pl.cdiv(n_io - n_first, n_groups)
    start([x_copy(i) for i in range(n_first)])
    start(head_copies(0))
    for i in range(n_first):
        x_copy(i).wait()
    for g in range(1, _COPIES_AHEAD):
        start(head_copies(g))
    start([x_copy(n_first + j) for j in range(per_group)])
    for i in range(n_first):
        transpose_in(i)
    early_h_ref[...] = _pack(normed(range(_LAG, _LAG + _EARLY)))

    def split_heads(g, c):
        tiles = []
        for t in range(c * _HEADS_PER_GROUP, (c + 1) * _HEADS_PER_GROUP):
            head, which = divmod(t, 3)
            words = stage_ref[g, 3 * (head // 2) + which]
            words = words & jnp.uint32(0xFFFF0000) if head % 2 else words << 16
            tiles.append(pltpu.bitcast(words, jnp.float32).astype(jnp.bfloat16))
        return jnp.concatenate(tiles, axis=1)

    @pl.loop(0, n_groups)
    def _load_group(g):
        tiles = [n_first + g * per_group + j for j in range(per_group)]
        for i in tiles:
            pl.when(i + per_group < n_io)(lambda i=i: x_copy(i + per_group).start())
        pl.when(g + _COPIES_AHEAD < n_groups)(lambda: start(head_copies(g + _COPIES_AHEAD)))
        pl.when(g == n_groups - _WO_COPY_LEAD)(lambda: start(wo_copies))
        pl.when(g == n_groups - _FFN_COPY_LEAD)(lambda: start(ffn_copies))
        for i in tiles:
            pl.when(i < n_io)(lambda i=i: x_copy(i).wait())
        for c in head_copies(g):
            c.wait()
        h = _unpack(early_h_ref[...])
        width = _HEADS_PER_GROUP * d_head
        weights = split_heads(g, 0)
        for c in range(3):
            following = split_heads(g, c + 1) if c < 2 else None
            cols = slice(c * width, (c + 1) * width)
            wqkv_ref[g, :, cols] = _pack(weights)
            early_ref[g, :_EARLY * seg // 2, cols] = _pack(_dot(h, weights).astype(jnp.bfloat16))
            weights = following
        for i in tiles:
            transpose_in(jnp.minimum(i, n_io - 1))

    for c in wo_copies:
        c.wait()

    mem0 = mem0_ref[...].astype(jnp.float32)
    mem1 = jax.lax.fori_loop(0, _LAG, first_step, mem0)
    for c in ffn_copies:
        c.wait()
    for g in range(n_groups):
        early_ref[g, _EARLY * seg // 2:, :] = _pack(spare_ref[g].astype(jnp.bfloat16))
    ffn_t, x = ffn_transposed(0)
    res_ref[n_tok:n_tok + 4 * seg, :] = x + ffn_t.T
    h_ref[:2 * n_mem, :] = jnp.concatenate([mem1, mem0], axis=0).astype(jnp.bfloat16)
    h_ref[2 * n_mem:, :] = normed([_LAG, n_seg])
    jax.lax.fori_loop(0, 2, functools.partial(double_step, early=True, with_ffn=False), mem0)
    jax.lax.fori_loop(2, _EARLY + 1, functools.partial(double_step, early=True), mem0)
    mem2 = jax.lax.fori_loop(_EARLY + 1, n_seg - _LAG, functools.partial(double_step, early=False),
                             mem0)

    n_done = (n_seg - _LAG - 8) * seg // _LANES + 1
    for i in range((_EARLY - 6) * seg // _LANES):
        transpose_out(i)
    start(out_copies[:n_done])
    last = 2 * n_seg - _LAG
    ffn_blocks = [n_seg - 2, n_seg - 1, last - 2, last - 1]
    mem2 = jax.lax.fori_loop(
        0, 2, lambda half, mem: single_step(last + half, mem, ffn_blocks, half), mem2)
    jax.lax.fori_loop(last + 2, 2 * n_seg, single_step, mem2)
    for i in range(n_done, n_io - 1):
        transpose_out(i)
        out_copies[i].start()
    ffn_t, x = ffn_transposed(last)
    tile_ref[n_io - 1] = (x.T + ffn_t).astype(tile_ref.dtype)
    out_copies[n_io - 1].start()
    for c in out_copies:
        c.wait()


@functools.partial(jax.jit, static_argnames=("A_seg_len",))
def pallas_interleave_layers__memory_aug_recurrent_mem_tr__glu_gated_swiglu__prompt_kernel(
    A_x: jax.Array,
    A_mem0: jax.Array,
    A_Wq: jax.Array,
    A_Wk: jax.Array,
    A_Wv: jax.Array,
    A_Wo: jax.Array,
    A_seg_len: int,
    B_x: jax.Array,
    B_w1: jax.Array,
    B_w3: jax.Array,
    B_w2: jax.Array,
):
    del B_x
    _, n_tok, d_model = A_x.shape
    n_mem = A_mem0.shape[1]
    _, n_heads, d_head = A_Wq.shape
    d_ff = B_w1.shape[1]
    n_groups = n_heads // _HEADS_PER_GROUP
    group_cols = 3 * d_head * _HEADS_PER_GROUP
    early_words = _EARLY * A_seg_len // 2
    hbm = pl.BlockSpec(memory_space=pltpu.HBM)
    out_t = pl.pallas_call(
        functools.partial(_kernel, seg=A_seg_len),
        out_shape=jax.ShapeDtypeStruct((d_model, n_tok), A_x.dtype),
        in_specs=[hbm] * 9,
        out_specs=hbm,
        scratch_shapes=[
            pltpu.VMEM((n_mem, d_model), A_mem0.dtype),
            pltpu.VMEM((n_tok // _LANES, d_model, _LANES), A_x.dtype),
            pltpu.VMEM((3 * n_tok, d_model), jnp.float32),
            pltpu.VMEM((2 * (n_mem + A_seg_len), d_model), jnp.bfloat16),
            pltpu.VMEM((early_words, d_model), jnp.uint32),
            pltpu.VMEM((n_groups, early_words + A_seg_len // 2, group_cols), jnp.uint32),
            pltpu.VMEM((n_groups, A_seg_len, group_cols), jnp.float32),
            pltpu.VMEM((n_groups, 3 * _HEADS_PER_GROUP // 2, d_model, d_head), jnp.uint32),
            pltpu.VMEM((n_groups, d_model // 2, group_cols), jnp.uint32),
            pltpu.VMEM((n_heads, d_model // 2, d_head), jnp.uint32),
            pltpu.VMEM((2, d_model // 2, d_ff // 2), jnp.uint32),
            pltpu.VMEM((2, d_model // 2, d_ff // 2), jnp.uint32),
            pltpu.VMEM((2, d_model // 2, d_ff // 2), jnp.uint32),
            pltpu.SemaphoreType.DMA((3 * n_heads // 2,)),
            pltpu.SemaphoreType.DMA((8,)),
            pltpu.SemaphoreType.DMA((n_tok // _LANES,)),
        ],
        compiler_params=pltpu.CompilerParams(vmem_limit_bytes=110 * 1024 * 1024),
    )(A_x.reshape(n_tok, d_model).T, A_mem0.reshape(n_mem, d_model), A_Wq, A_Wk, A_Wv,
      A_Wo.transpose(0, 2, 1), B_w1, B_w3, B_w2.T)
    return out_t.T.reshape(A_x.shape)
```

```python
import functools
import math

import jax
import jax.numpy as jnp
import jax.experimental.pallas as pl
import jax.experimental.pallas.tpu as pltpu

_EPS = 1e-05
_MASKED = -1000000000.0
_LOG2E = math.log2(math.e)
_LANES = 128
_LAG = 4
_EARLY = 16
_HEADS_PER_GROUP = 4
_FFN_CHUNK = 768
_COPIES_AHEAD = 2
_WO_COPY_LEAD = 2
_FFN_COPY_LEAD = 2
_ORDER = (
    "P0 P1 S0 P2 V0 G0 S1 S2 P3 V1 O0 G1 S3 V2 P4 O1 P5 V3 O2 S4 P6 V4 G2 S5 P7 S6 O3 V5 "
    "O4 S7 V6 D0 O5 V7 O6 O7")
_ORDER_EARLY = (
    "P0 P1 S0 P2 V0 G0 S1 S2 P3 V1 O0 G1 O1 S3 V2 P4 P5 V3 S4 P6 O2 G2 P7 S5 V4 S6 O3 V5 "
    "O4 S7 V6 D0 O5 V7 O6 O7")
_ORDER_ATTENTION = (
    "P0 P1 S0 P2 S1 V0 P3 V1 O0 S2 P4 V2 O1 S3 P5 S4 V3 O2 S5 P6 O3 V4 S6 V5 P7 O4 S7 V6 "
    "O5 V7 O6 O7")


def _layernorm(x):
    m = jnp.mean(x, axis=-1, keepdims=True)
    d = x - m
    v = jnp.mean(d * d, axis=-1, keepdims=True)
    return d * jax.lax.rsqrt(v + _EPS)


def _dot(a, b):
    return jnp.dot(a, b, preferred_element_type=jnp.float32)


def _dot_nt(a, b):
    return jax.lax.dot_general(a, b, (((1,), (1,)), ((), ())),
                               preferred_element_type=jnp.float32)


def _pack(x):
    return pltpu.bitcast(x, jnp.uint32)


def _unpack(words):
    return pltpu.bitcast(words, jnp.bfloat16)


def _attention_masks(n_layers, n_mem, seg):
    rows = n_layers * (n_mem + seg)
    i = jax.lax.broadcasted_iota(jnp.int32, (rows, rows), 0)
    j = jax.lax.broadcasted_iota(jnp.int32, (rows, rows), 1)
    visible = (i < n_layers * n_mem) | (i >= j)
    if n_layers == 1:
        return visible, _MASKED * _LOG2E

    def second_layer(r):
        return ((r >= n_mem) & (r < 2 * n_mem)) | (r >= 2 * n_mem + seg)

    same = second_layer(i) == second_layer(j)
    fill = jnp.where(same, _MASKED * _LOG2E, -jnp.inf).astype(jnp.float32)
    return same & visible, fill


def _kernel(xt_hbm, mem0_hbm, wq_hbm, wk_hbm, wv_hbm, wot_hbm, w1_hbm, w3_hbm, w2t_hbm,
            outt_hbm, mem0_ref, tile_ref, res_ref, h_ref, early_h_ref, early_ref, spare_ref,
            stage_ref, wqkv_ref, wot_ref,
            w1_ref, w3_ref, w2t_ref, stage_sem, weight_sem, tile_sem, *, seg):
    d_model, n_tok = xt_hbm.shape
    n_mem = mem0_ref.shape[0]
    _, n_heads, d_head = wq_hbm.shape
    n_groups = n_heads // _HEADS_PER_GROUP
    half_ff = w2t_ref.shape[2]
    n_chunks = half_ff // _FFN_CHUNK
    n_seg = n_tok // seg
    n_io = n_tok // _LANES
    score_scale = d_head ** -0.5 * _LOG2E

    def block(r):
        return pl.ds(pl.multiple_of(r * seg, seg), seg)

    def load_blocks(blocks):
        return jnp.concatenate([res_ref[block(r), :] for r in blocks], axis=0)

    def store_blocks(blocks, value):
        for i, r in enumerate(blocks):
            res_ref[block(r), :] = value[i * seg:(i + 1) * seg]

    def normed(blocks):
        return _layernorm(load_blocks(blocks)).astype(jnp.bfloat16)

    def transpose_out(i):
        rows = pl.ds(pl.multiple_of(2 * n_tok + i * _LANES, _LANES), _LANES)
        tile_ref[i] = res_ref[rows, :].T.astype(tile_ref.dtype)

    def gated(hn, half, c):
        cols = slice(c * _FFN_CHUNK, (c + 1) * _FFN_CHUNK)
        both = _dot(hn, _unpack(
            jnp.concatenate([w1_ref[half, :, cols], w3_ref[half, :, cols]], axis=1)))
        gate, up = both[:, :_FFN_CHUNK], both[:, _FFN_CHUNK:]
        return (gate * jax.nn.sigmoid(gate) * up).astype(jnp.bfloat16)

    def mix(order, project, attn_blocks, ffn_blocks, half):
        n_layers = len(attn_blocks)
        visible, fill = _attention_masks(n_layers, n_mem, seg)
        if ffn_blocks:
            hn = normed(ffn_blocks)
        qkv, probs, heads, acts, out, y = {}, {}, {}, [], None, None

        def part(g, head, which):
            col = (3 * head + which) * d_head
            return qkv[g][:, col:col + d_head]

        for name in order.split():
            stage, g = name[0], int(name[1:])
            if stage in "GD" and not ffn_blocks:
                continue
            if stage == "P":
                qkv[g] = project(g)
            elif stage == "S":
                probs[g] = []
                for s in [_dot_nt(part(g, i, 0), part(g, i, 1)) for i in range(_HEADS_PER_GROUP)]:
                    s = jnp.where(visible, s * score_scale, fill)
                    p = jnp.exp2(s - jnp.max(s, axis=-1, keepdims=True))
                    inv = 1.0 / jnp.sum(p, axis=-1, keepdims=True)
                    probs[g].append((p.astype(jnp.bfloat16), inv))
            elif stage == "V":
                heads[g] = [(_dot(p, part(g, i, 2)) * inv).astype(jnp.bfloat16)
                            for i, (p, inv) in enumerate(probs[g])]
            elif stage == "O":
                wo = [wot_ref[g * _HEADS_PER_GROUP + i] for i in range(_HEADS_PER_GROUP)]
                o = _dot_nt(jnp.concatenate(heads[g], axis=1),
                            _unpack(jnp.concatenate(wo, axis=1)))
                out = o if out is None else out + o
            elif stage == "G":
                acts.append(gated(hn, half, g))
            elif stage == "D":
                y = _dot_nt(_unpack(w2t_ref[half]), jnp.concatenate(acts, axis=1)).T
                y = y + load_blocks([r + half * n_seg for r in ffn_blocks])
        if ffn_blocks:
            store_blocks([r + n_seg for r in ffn_blocks], y)
        store_blocks(attn_blocks, load_blocks(attn_blocks) + out[n_layers * n_mem:])
        return out[:n_layers * n_mem], y

    def projector(h):
        return lambda g: _dot(h, _unpack(wqkv_ref[g])).astype(jnp.bfloat16)

    def single_step(r, mem, ffn_blocks=(), half=None):
        h = jnp.concatenate([mem, _layernorm(load_blocks([r]))], axis=0)
        order = _ORDER_EARLY if ffn_blocks else _ORDER_ATTENTION
        return mix(order, projector(h.astype(jnp.bfloat16)), [r], ffn_blocks, half)[0]

    def first_step(r, mem):
        spare = seg // _LAG
        rows = pl.ds(pl.multiple_of(r * spare, spare), spare)
        ahead = res_ref[pl.ds(pl.multiple_of((_LAG + _EARLY) * seg + r * spare, spare), spare), :]
        x = jnp.concatenate([load_blocks([r]), ahead], axis=0)
        h = jnp.concatenate([mem, _layernorm(x)], axis=0).astype(jnp.bfloat16)

        def project(g):
            qkv = _dot(h, _unpack(wqkv_ref[g]))
            spare_ref[g, rows, :] = qkv[n_mem + seg:]
            return qkv[:n_mem + seg].astype(jnp.bfloat16)

        return mix(_ORDER_ATTENTION, project, [r], (), None)[0]

    def ffn_transposed(first):
        x = res_ref[first * seg:(first + 4) * seg, :]
        hn = _layernorm(x).astype(jnp.bfloat16)
        halves = [
            _dot_nt(_unpack(w2t_ref[half]),
                    jnp.concatenate([gated(hn, half, c) for c in range(n_chunks)], axis=1))
            for half in range(2)]
        return halves[0] + halves[1], x

    def double_step(b, _, *, early, with_ffn=True):
        half = b % 2
        f1, f2 = b - half + _LAG - 2, n_seg + b - half - 2
        if early:
            rest = projector(jnp.concatenate(
                [h_ref[:2 * n_mem, :], h_ref[2 * n_mem + seg:, :]], axis=0))
            rows = pl.ds(pl.multiple_of(b * (seg // 2), seg // 2), seg // 2)

            def project(g):
                qkv = rest(g)
                known = _unpack(early_ref[g, rows, :])
                return jnp.concatenate([qkv[:2 * n_mem], known, qkv[2 * n_mem:]], axis=0)
        else:
            project = projector(h_ref[...])
            transpose_out((b - 7) * seg // _LANES)
        h1 = normed([jnp.minimum(b + 1 + _LAG, n_seg - 1)])
        x2 = load_blocks([n_seg + b + 1 - half])
        order = _ORDER_EARLY if early and with_ffn else _ORDER
        mems, y = mix(order, project, [b + _LAG, n_seg + b],
                      [f1, f1 + 1, f2, f2 + 1] if with_ffn else [], half)
        x2 = jnp.where(half == 1, y[:seg], x2) if with_ffn else load_blocks([n_seg + b + 1])
        h_ref[:2 * n_mem, :] = mems.astype(jnp.bfloat16)
        h_ref[2 * n_mem:2 * n_mem + seg, :] = h1
        h_ref[2 * n_mem + seg:, :] = _layernorm(x2).astype(jnp.bfloat16)
        return mems[n_mem:]

    pairs = _HEADS_PER_GROUP // 2

    def head_copies(g):
        return [pltpu.make_async_copy(w.bitcast(jnp.uint32).at[:, g * pairs + p, :],
                                      stage_ref.at[g, 3 * p + i], stage_sem.at[3 * (g * pairs + p) + i])
                for p in range(pairs) for i, w in enumerate((wq_hbm, wk_hbm, wv_hbm))]

    def x_copy(i):
        cols = pl.ds(pl.multiple_of(i * _LANES, _LANES), _LANES)
        return pltpu.make_async_copy(xt_hbm.at[:, cols], tile_ref.at[i], tile_sem.at[i])

    wo_copies = [pltpu.make_async_copy(wot_hbm.bitcast(jnp.uint32), wot_ref, weight_sem.at[0]),
                 pltpu.make_async_copy(mem0_hbm, mem0_ref, weight_sem.at[7])]
    ffn_copies = [
        pltpu.make_async_copy(src.bitcast(jnp.uint32).at[:, pl.ds(half * half_ff, half_ff)],
                              dst.at[half], weight_sem.at[1 + 2 * i + half])
        for half in range(2)
        for i, (src, dst) in enumerate(((w1_hbm, w1_ref), (w3_hbm, w3_ref), (w2t_hbm, w2t_ref)))]

    out_copies = [
        pltpu.make_async_copy(tile_ref.at[i],
                              outt_hbm.at[:, pl.ds(i * _LANES, _LANES)], tile_sem.at[i])
        for i in range(n_io)]

    def transpose_in(i):
        rows = pl.ds(pl.multiple_of(i * _LANES, _LANES), _LANES)
        res_ref[rows, :] = tile_ref[i].astype(jnp.float32).T

    def start(copies):
        for c in copies:
            c.start()

    n_first = pl.cdiv((_LAG + _EARLY) * seg, _LANES)
    per_group = pl.cdiv(n_io - n_first, n_groups)
    start([x_copy(i) for i in range(n_first)])
    start(head_copies(0))
    for i in range(n_first):
        x_copy(i).wait()
    for g in range(1, _COPIES_AHEAD):
        start(head_copies(g))
    start([x_copy(n_first + j) for j in range(per_group)])
    for i in range(n_first):
        transpose_in(i)
    early_h_ref[...] = _pack(normed(range(_LAG, _LAG + _EARLY)))

    def split_heads(g, c):
        tiles = []
        for t in range(c * _HEADS_PER_GROUP, (c + 1) * _HEADS_PER_GROUP):
            head, which = divmod(t, 3)
            words = stage_ref[g, 3 * (head // 2) + which]
            words = words & jnp.uint32(0xFFFF0000) if head % 2 else words << 16
            tiles.append(pltpu.bitcast(words, jnp.float32).astype(jnp.bfloat16))
        return jnp.concatenate(tiles, axis=1)

    @pl.loop(0, n_groups)
    def _load_group(g):
        tiles = [n_first + g * per_group + j for j in range(per_group)]
        for i in tiles:
            pl.when(i + per_group < n_io)(lambda i=i: x_copy(i + per_group).start())
        pl.when(g + _COPIES_AHEAD < n_groups)(lambda: start(head_copies(g + _COPIES_AHEAD)))
        pl.when(g == n_groups - _WO_COPY_LEAD)(lambda: start(wo_copies))
        pl.when(g == n_groups - _FFN_COPY_LEAD)(lambda: start(ffn_copies))
        for i in tiles:
            pl.when(i < n_io)(lambda i=i: x_copy(i).wait())
        for c in head_copies(g):
            c.wait()
        h = _unpack(early_h_ref[...])
        width = _HEADS_PER_GROUP * d_head
        weights = split_heads(g, 0)
        for c in range(3):
            following = split_heads(g, c + 1) if c < 2 else None
            cols = slice(c * width, (c + 1) * width)
            wqkv_ref[g, :, cols] = _pack(weights)
            early_ref[g, :_EARLY * seg // 2, cols] = _pack(_dot(h, weights).astype(jnp.bfloat16))
            weights = following
        for i in tiles:
            transpose_in(jnp.minimum(i, n_io - 1))

    for c in wo_copies:
        c.wait()

    mem0 = mem0_ref[...].astype(jnp.float32)
    mem1 = jax.lax.fori_loop(0, _LAG, first_step, mem0)
    for c in ffn_copies:
        c.wait()
    for g in range(n_groups):
        early_ref[g, _EARLY * seg // 2:, :] = _pack(spare_ref[g].astype(jnp.bfloat16))
    ffn_t, x = ffn_transposed(0)
    res_ref[n_tok:n_tok + 4 * seg, :] = x + ffn_t.T
    h_ref[:2 * n_mem, :] = jnp.concatenate([mem1, mem0], axis=0).astype(jnp.bfloat16)
    h_ref[2 * n_mem:, :] = normed([_LAG, n_seg])
    jax.lax.fori_loop(0, 2, functools.partial(double_step, early=True, with_ffn=False), mem0)
    jax.lax.fori_loop(2, _EARLY + 1, functools.partial(double_step, early=True), mem0)
    mem2 = jax.lax.fori_loop(_EARLY + 1, n_seg - _LAG, functools.partial(double_step, early=False),
                             mem0)

    n_done = (n_seg - _LAG - 8) * seg // _LANES + 1
    for i in range((_EARLY - 6) * seg // _LANES):
        transpose_out(i)
    start(out_copies[:n_done])
    last = 2 * n_seg - _LAG
    ffn_blocks = [n_seg - 2, n_seg - 1, last - 2, last - 1]
    mem2 = jax.lax.fori_loop(
        0, 2, lambda half, mem: single_step(last + half, mem, ffn_blocks, half), mem2)
    jax.lax.fori_loop(last + 2, 2 * n_seg, single_step, mem2)
    for i in range(n_done, n_io - 1):
        transpose_out(i)
        out_copies[i].start()
    ffn_t, x = ffn_transposed(last)
    tile_ref[n_io - 1] = (x.T + ffn_t).astype(tile_ref.dtype)
    out_copies[n_io - 1].start()
    for c in out_copies:
        c.wait()


@functools.partial(jax.jit, static_argnames=("A_seg_len",))
def pallas_interleave_layers__memory_aug_recurrent_mem_tr__glu_gated_swiglu__prompt_kernel(
    A_x: jax.Array,
    A_mem0: jax.Array,
    A_Wq: jax.Array,
    A_Wk: jax.Array,
    A_Wv: jax.Array,
    A_Wo: jax.Array,
    A_seg_len: int,
    B_x: jax.Array,
    B_w1: jax.Array,
    B_w3: jax.Array,
    B_w2: jax.Array,
):
    del B_x
    _, n_tok, d_model = A_x.shape
    n_mem = A_mem0.shape[1]
    _, n_heads, d_head = A_Wq.shape
    d_ff = B_w1.shape[1]
    n_groups = n_heads // _HEADS_PER_GROUP
    group_cols = 3 * d_head * _HEADS_PER_GROUP
    early_words = _EARLY * A_seg_len // 2
    hbm = pl.BlockSpec(memory_space=pltpu.HBM)
    out_t = pl.pallas_call(
        functools.partial(_kernel, seg=A_seg_len),
        out_shape=jax.ShapeDtypeStruct((d_model, n_tok), A_x.dtype),
        in_specs=[hbm] * 9,
        out_specs=hbm,
        scratch_shapes=[
            pltpu.VMEM((n_mem, d_model), A_mem0.dtype),
            pltpu.VMEM((n_tok // _LANES, d_model, _LANES), A_x.dtype),
            pltpu.VMEM((3 * n_tok, d_model), jnp.float32),
            pltpu.VMEM((2 * (n_mem + A_seg_len), d_model), jnp.bfloat16),
            pltpu.VMEM((early_words, d_model), jnp.uint32),
            pltpu.VMEM((n_groups, early_words + A_seg_len // 2, group_cols), jnp.uint32),
            pltpu.VMEM((n_groups, A_seg_len, group_cols), jnp.float32),
            pltpu.VMEM((n_groups, 3 * _HEADS_PER_GROUP // 2, d_model, d_head), jnp.uint32),
            pltpu.VMEM((n_groups, d_model // 2, group_cols), jnp.uint32),
            pltpu.VMEM((n_heads, d_model // 2, d_head), jnp.uint32),
            pltpu.VMEM((2, d_model // 2, d_ff // 2), jnp.uint32),
            pltpu.VMEM((2, d_model // 2, d_ff // 2), jnp.uint32),
            pltpu.VMEM((2, d_model // 2, d_ff // 2), jnp.uint32),
            pltpu.SemaphoreType.DMA((3 * n_heads // 2,)),
            pltpu.SemaphoreType.DMA((8,)),
            pltpu.SemaphoreType.DMA((n_tok // _LANES,)),
        ],
        compiler_params=pltpu.CompilerParams(vmem_limit_bytes=110 * 1024 * 1024),
    )(A_x.reshape(n_tok, d_model).T, A_mem0.reshape(n_mem, d_model), A_Wq, A_Wk, A_Wv,
      A_Wo.transpose(0, 2, 1), B_w1, B_w3, B_w2.T)
    return out_t.T.reshape(A_x.shape)
```

```python
import functools
import math

import jax
import jax.numpy as jnp
import jax.experimental.pallas as pl
import jax.experimental.pallas.tpu as pltpu

_EPS = 1e-05
_MASKED = -1000000000.0
_LOG2E = math.log2(math.e)
_LANES = 128
_LAG = 4
_EARLY = 16
_HEADS_PER_GROUP = 4
_FFN_CHUNK = 768
_COPIES_AHEAD = 2
_WO_COPY_LEAD = 2
_FFN_COPY_LEAD = 2
_ORDER = (
    "P0 P1 S0 P2 V0 G0 S1 S2 P3 V1 O0 G1 S3 V2 P4 O1 P5 V3 O2 S4 P6 V4 G2 S5 P7 S6 O3 V5 "
    "O4 S7 V6 D0 O5 V7 O6 O7")
_ORDER_EARLY = (
    "P0 P1 S0 P2 V0 G0 S1 S2 P3 V1 O0 G1 O1 S3 V2 P4 P5 V3 S4 P6 O2 G2 P7 S5 V4 S6 O3 V5 "
    "O4 S7 V6 D0 O5 V7 O6 O7")
_ORDER_ATTENTION = (
    "P0 P1 S0 P2 S1 V0 P3 V1 O0 S2 P4 V2 O1 S3 P5 S4 V3 O2 S5 P6 O3 V4 S6 V5 P7 O4 S7 V6 "
    "O5 V7 O6 O7")


def _layernorm(x):
    m = jnp.mean(x, axis=-1, keepdims=True)
    d = x - m
    v = jnp.mean(d * d, axis=-1, keepdims=True)
    return d * jax.lax.rsqrt(v + _EPS)


def _dot(a, b):
    return jnp.dot(a, b, preferred_element_type=jnp.float32)


def _dot_nt(a, b):
    return jax.lax.dot_general(a, b, (((1,), (1,)), ((), ())),
                               preferred_element_type=jnp.float32)


def _pack(x):
    return pltpu.bitcast(x, jnp.uint32)


def _unpack(words):
    return pltpu.bitcast(words, jnp.bfloat16)


def _attention_masks(n_layers, n_mem, seg):
    rows = n_layers * (n_mem + seg)
    i = jax.lax.broadcasted_iota(jnp.int32, (rows, rows), 0)
    j = jax.lax.broadcasted_iota(jnp.int32, (rows, rows), 1)
    visible = (i < n_layers * n_mem) | (i >= j)
    if n_layers == 1:
        return visible, _MASKED * _LOG2E

    def second_layer(r):
        return ((r >= n_mem) & (r < 2 * n_mem)) | (r >= 2 * n_mem + seg)

    same = second_layer(i) == second_layer(j)
    fill = jnp.where(same, _MASKED * _LOG2E, -jnp.inf).astype(jnp.float32)
    return same & visible, fill


def _kernel(xt_hbm, mem0_hbm, wq_hbm, wk_hbm, wv_hbm, wot_hbm, w1_hbm, w3_hbm, w2t_hbm,
            outt_hbm, mem0_ref, tile_ref, res_ref, h_ref, early_h_ref, early_ref, spare_ref,
            stage_ref, wqkv_ref, wot_ref,
            w1_ref, w3_ref, w2t_ref, stage_sem, weight_sem, tile_sem, *, seg):
    d_model, n_tok = xt_hbm.shape
    n_mem = mem0_ref.shape[0]
    _, n_heads, d_head = wq_hbm.shape
    n_groups = n_heads // _HEADS_PER_GROUP
    half_ff = w2t_ref.shape[2]
    n_chunks = half_ff // _FFN_CHUNK
    n_seg = n_tok // seg
    n_io = n_tok // _LANES
    score_scale = d_head ** -0.5 * _LOG2E

    def block(r):
        return pl.ds(pl.multiple_of(r * seg, seg), seg)

    def load_blocks(blocks):
        return jnp.concatenate([res_ref[block(r), :] for r in blocks], axis=0)

    def store_blocks(blocks, value):
        for i, r in enumerate(blocks):
            res_ref[block(r), :] = value[i * seg:(i + 1) * seg]

    def normed(blocks):
        return _layernorm(load_blocks(blocks)).astype(jnp.bfloat16)

    def transpose_out(i):
        rows = pl.ds(pl.multiple_of(2 * n_tok + i * _LANES, _LANES), _LANES)
        tile_ref[i] = res_ref[rows, :].T.astype(tile_ref.dtype)

    def gated(hn, half, c):
        cols = slice(c * _FFN_CHUNK, (c + 1) * _FFN_CHUNK)
        both = _dot(hn, _unpack(
            jnp.concatenate([w1_ref[half, :, cols], w3_ref[half, :, cols]], axis=1)))
        gate, up = both[:, :_FFN_CHUNK], both[:, _FFN_CHUNK:]
        return (gate * jax.nn.sigmoid(gate) * up).astype(jnp.bfloat16)

    def mix(order, project, attn_blocks, ffn_blocks, half):
        n_layers = len(attn_blocks)
        visible, fill = _attention_masks(n_layers, n_mem, seg)
        if ffn_blocks:
            hn = normed(ffn_blocks)
        qkv, probs, heads, acts, out, y = {}, {}, {}, [], None, None

        def part(g, head, which):
            col = (3 * head + which) * d_head
            return qkv[g][:, col:col + d_head]

        for name in order.split():
            stage, g = name[0], int(name[1:])
            if stage in "GD" and not ffn_blocks:
                continue
            if stage == "P":
                qkv[g] = project(g)
            elif stage == "S":
                probs[g] = []
                for s in [_dot_nt(part(g, i, 0), part(g, i, 1)) for i in range(_HEADS_PER_GROUP)]:
                    s = jnp.where(visible, s * score_scale, fill)
                    p = jnp.exp2(s - jnp.max(s, axis=-1, keepdims=True))
                    inv = 1.0 / jnp.sum(p, axis=-1, keepdims=True)
                    probs[g].append((p.astype(jnp.bfloat16), inv))
            elif stage == "V":
                heads[g] = [(_dot(p, part(g, i, 2)) * inv).astype(jnp.bfloat16)
                            for i, (p, inv) in enumerate(probs[g])]
            elif stage == "O":
                wo = [wot_ref[g * _HEADS_PER_GROUP + i] for i in range(_HEADS_PER_GROUP)]
                o = _dot_nt(jnp.concatenate(heads[g], axis=1),
                            _unpack(jnp.concatenate(wo, axis=1)))
                out = o if out is None else out + o
            elif stage == "G":
                acts.append(gated(hn, half, g))
            elif stage == "D":
                y = _dot_nt(_unpack(w2t_ref[half]), jnp.concatenate(acts, axis=1)).T
                y = y + load_blocks([r + half * n_seg for r in ffn_blocks])
        if ffn_blocks:
            store_blocks([r + n_seg for r in ffn_blocks], y)
        store_blocks(attn_blocks, load_blocks(attn_blocks) + out[n_layers * n_mem:])
        return out[:n_layers * n_mem], y

    def projector(h):
        return lambda g: _dot(h, _unpack(wqkv_ref[g])).astype(jnp.bfloat16)

    def single_step(r, mem, ffn_blocks=(), half=None):
        h = jnp.concatenate([mem, _layernorm(load_blocks([r]))], axis=0)
        order = _ORDER_EARLY if ffn_blocks else _ORDER_ATTENTION
        return mix(order, projector(h.astype(jnp.bfloat16)), [r], ffn_blocks, half)[0]

    def first_step(r, mem):
        spare = seg // _LAG
        rows = pl.ds(pl.multiple_of(r * spare, spare), spare)
        ahead = res_ref[pl.ds(pl.multiple_of((_LAG + _EARLY) * seg + r * spare, spare), spare), :]
        x = jnp.concatenate([load_blocks([r]), ahead], axis=0)
        h = jnp.concatenate([mem, _layernorm(x)], axis=0).astype(jnp.bfloat16)

        def project(g):
            qkv = _dot(h, _unpack(wqkv_ref[g]))
            spare_ref[g, rows, :] = qkv[n_mem + seg:]
            return qkv[:n_mem + seg].astype(jnp.bfloat16)

        return mix(_ORDER_ATTENTION, project, [r], (), None)[0]

    def ffn_transposed(first):
        x = res_ref[first * seg:(first + 4) * seg, :]
        hn = _layernorm(x).astype(jnp.bfloat16)
        halves = [
            _dot_nt(_unpack(w2t_ref[half]),
                    jnp.concatenate([gated(hn, half, c) for c in range(n_chunks)], axis=1))
            for half in range(2)]
        return halves[0] + halves[1], x

    def double_step(b, _, *, early, with_ffn=True):
        half = b % 2
        f1, f2 = b - half + _LAG - 2, n_seg + b - half - 2
        if early:
            rest = projector(jnp.concatenate(
                [h_ref[:2 * n_mem, :], h_ref[2 * n_mem + seg:, :]], axis=0))
            rows = pl.ds(pl.multiple_of(b * (seg // 2), seg // 2), seg // 2)

            def project(g):
                qkv = rest(g)
                known = _unpack(early_ref[g, rows, :])
                return jnp.concatenate([qkv[:2 * n_mem], known, qkv[2 * n_mem:]], axis=0)
        else:
            project = projector(h_ref[...])
            transpose_out((b - 7) * seg // _LANES)
        h1 = normed([jnp.minimum(b + 1 + _LAG, n_seg - 1)])
        x2 = load_blocks([n_seg + b + 1 - half])
        order = _ORDER_EARLY if early and with_ffn else _ORDER
        mems, y = mix(order, project, [b + _LAG, n_seg + b],
                      [f1, f1 + 1, f2, f2 + 1] if with_ffn else [], half)
        x2 = jnp.where(half == 1, y[:seg], x2) if with_ffn else load_blocks([n_seg + b + 1])
        h_ref[:2 * n_mem, :] = mems.astype(jnp.bfloat16)
        h_ref[2 * n_mem:2 * n_mem + seg, :] = h1
        h_ref[2 * n_mem + seg:, :] = _layernorm(x2).astype(jnp.bfloat16)
        return mems[n_mem:]

    pairs = _HEADS_PER_GROUP // 2

    def head_copies(g):
        return [pltpu.make_async_copy(w.bitcast(jnp.uint32).at[:, g * pairs + p, :],
                                      stage_ref.at[g, 3 * p + i],
                                      stage_sem.at[3 * (g * pairs + p) + i])
                for p in range(pairs) for i, w in enumerate((wq_hbm, wk_hbm, wv_hbm))]

    def x_copy(i):
        cols = pl.ds(pl.multiple_of(i * _LANES, _LANES), _LANES)
        return pltpu.make_async_copy(xt_hbm.at[:, cols], tile_ref.at[i], tile_sem.at[i])

    wo_copies = [pltpu.make_async_copy(wot_hbm.bitcast(jnp.uint32), wot_ref, weight_sem.at[0]),
                 pltpu.make_async_copy(mem0_hbm, mem0_ref, weight_sem.at[7])]
    ffn_copies = [
        pltpu.make_async_copy(src.bitcast(jnp.uint32).at[:, pl.ds(half * half_ff, half_ff)],
                              dst.at[half], weight_sem.at[1 + 2 * i + half])
        for half in range(2)
        for i, (src, dst) in enumerate(((w1_hbm, w1_ref), (w3_hbm, w3_ref), (w2t_hbm, w2t_ref)))]

    out_copies = [
        pltpu.make_async_copy(tile_ref.at[i],
                              outt_hbm.at[:, pl.ds(i * _LANES, _LANES)], tile_sem.at[i])
        for i in range(n_io)]

    def transpose_in(i):
        rows = pl.ds(pl.multiple_of(i * _LANES, _LANES), _LANES)
        res_ref[rows, :] = tile_ref[i].astype(jnp.float32).T

    def start(copies):
        for c in copies:
            c.start()

    n_first = pl.cdiv((_LAG + _EARLY) * seg, _LANES)
    per_group = pl.cdiv(n_io - n_first, n_groups)
    start([x_copy(i) for i in range(n_first)])
    start(head_copies(0))
    for i in range(n_first):
        x_copy(i).wait()
    for g in range(1, _COPIES_AHEAD):
        start(head_copies(g))
    start([x_copy(n_first + j) for j in range(per_group)])
    for i in range(n_first):
        transpose_in(i)
    early_h_ref[...] = _pack(normed(range(_LAG, _LAG + _EARLY)))

    def split_heads(g, c):
        tiles = []
        for t in range(c * _HEADS_PER_GROUP, (c + 1) * _HEADS_PER_GROUP):
            head, which = divmod(t, 3)
            words = stage_ref[g, 3 * (head // 2) + which]
            words = words & jnp.uint32(0xFFFF0000) if head % 2 else words << 16
            tiles.append(pltpu.bitcast(words, jnp.float32).astype(jnp.bfloat16))
        return jnp.concatenate(tiles, axis=1)

    @pl.loop(0, n_groups)
    def _load_group(g):
        tiles = [n_first + g * per_group + j for j in range(per_group)]
        for i in tiles:
            pl.when(i + per_group < n_io)(lambda i=i: x_copy(i + per_group).start())
        pl.when(g + _COPIES_AHEAD < n_groups)(lambda: start(head_copies(g + _COPIES_AHEAD)))
        pl.when(g == n_groups - _WO_COPY_LEAD)(lambda: start(wo_copies))
        pl.when(g == n_groups - _FFN_COPY_LEAD)(lambda: start(ffn_copies))
        for i in tiles:
            pl.when(i < n_io)(lambda i=i: x_copy(i).wait())
        for c in head_copies(g):
            c.wait()
        h = _unpack(early_h_ref[...])
        width = _HEADS_PER_GROUP * d_head
        weights = split_heads(g, 0)
        for c in range(3):
            following = split_heads(g, c + 1) if c < 2 else None
            cols = slice(c * width, (c + 1) * width)
            wqkv_ref[g, :, cols] = _pack(weights)
            early_ref[g, :_EARLY * seg // 2, cols] = _pack(_dot(h, weights).astype(jnp.bfloat16))
            weights = following
        for i in tiles:
            transpose_in(jnp.minimum(i, n_io - 1))

    for c in wo_copies:
        c.wait()

    mem0 = mem0_ref[...].astype(jnp.float32)
    mem1 = jax.lax.fori_loop(0, _LAG, first_step, mem0)
    for c in ffn_copies:
        c.wait()
    for g in range(n_groups):
        early_ref[g, _EARLY * seg // 2:, :] = _pack(spare_ref[g].astype(jnp.bfloat16))
    ffn_t, x = ffn_transposed(0)
    res_ref[n_tok:n_tok + 4 * seg, :] = x + ffn_t.T
    h_ref[:2 * n_mem, :] = jnp.concatenate([mem1, mem0], axis=0).astype(jnp.bfloat16)
    h_ref[2 * n_mem:, :] = normed([_LAG, n_seg])
    jax.lax.fori_loop(0, 2, functools.partial(double_step, early=True, with_ffn=False), mem0)
    jax.lax.fori_loop(2, _EARLY + 1, functools.partial(double_step, early=True), mem0)
    mem2 = jax.lax.fori_loop(_EARLY + 1, n_seg - _LAG, functools.partial(double_step, early=False),
                             mem0)

    n_done = (n_seg - _LAG - 8) * seg // _LANES + 1
    for i in range((_EARLY - 6) * seg // _LANES):
        transpose_out(i)
    start(out_copies[:n_done])
    last = 2 * n_seg - _LAG
    ffn_blocks = [n_seg - 2, n_seg - 1, last - 2, last - 1]
    mem2 = jax.lax.fori_loop(
        0, 2, lambda half, mem: single_step(last + half, mem, ffn_blocks, half), mem2)
    jax.lax.fori_loop(last + 2, 2 * n_seg, single_step, mem2)
    for i in range(n_done, n_io - 1):
        transpose_out(i)
        out_copies[i].start()
    ffn_t, x = ffn_transposed(last)
    tile_ref[n_io - 1] = (x.T + ffn_t).astype(tile_ref.dtype)
    out_copies[n_io - 1].start()
    for c in out_copies:
        c.wait()


@functools.partial(jax.jit, static_argnames=("A_seg_len",))
def pallas_interleave_layers__memory_aug_recurrent_mem_tr__glu_gated_swiglu__prompt_kernel(
    A_x: jax.Array,
    A_mem0: jax.Array,
    A_Wq: jax.Array,
    A_Wk: jax.Array,
    A_Wv: jax.Array,
    A_Wo: jax.Array,
    A_seg_len: int,
    B_x: jax.Array,
    B_w1: jax.Array,
    B_w3: jax.Array,
    B_w2: jax.Array,
):
    del B_x
    _, n_tok, d_model = A_x.shape
    n_mem = A_mem0.shape[1]
    _, n_heads, d_head = A_Wq.shape
    d_ff = B_w1.shape[1]
    assert A_x.shape[0] == 1 and 4 * A_seg_len == _LANES and A_seg_len // _LAG == n_mem == 8
    assert n_heads == 8 * _HEADS_PER_GROUP and d_ff == 6 * _FFN_CHUNK
    n_groups = n_heads // _HEADS_PER_GROUP
    group_cols = 3 * d_head * _HEADS_PER_GROUP
    early_words = _EARLY * A_seg_len // 2
    hbm = pl.BlockSpec(memory_space=pltpu.HBM)
    out_t = pl.pallas_call(
        functools.partial(_kernel, seg=A_seg_len),
        out_shape=jax.ShapeDtypeStruct((d_model, n_tok), A_x.dtype),
        in_specs=[hbm] * 9,
        out_specs=hbm,
        scratch_shapes=[
            pltpu.VMEM((n_mem, d_model), A_mem0.dtype),
            pltpu.VMEM((n_tok // _LANES, d_model, _LANES), A_x.dtype),
            pltpu.VMEM((3 * n_tok, d_model), jnp.float32),
            pltpu.VMEM((2 * (n_mem + A_seg_len), d_model), jnp.bfloat16),
            pltpu.VMEM((early_words, d_model), jnp.uint32),
            pltpu.VMEM((n_groups, early_words + A_seg_len // 2, group_cols), jnp.uint32),
            pltpu.VMEM((n_groups, A_seg_len, group_cols), jnp.float32),
            pltpu.VMEM((n_groups, 3 * _HEADS_PER_GROUP // 2, d_model, d_head), jnp.uint32),
            pltpu.VMEM((n_groups, d_model // 2, group_cols), jnp.uint32),
            pltpu.VMEM((n_heads, d_model // 2, d_head), jnp.uint32),
            pltpu.VMEM((2, d_model // 2, d_ff // 2), jnp.uint32),
            pltpu.VMEM((2, d_model // 2, d_ff // 2), jnp.uint32),
            pltpu.VMEM((2, d_model // 2, d_ff // 2), jnp.uint32),
            pltpu.SemaphoreType.DMA((3 * n_heads // 2,)),
            pltpu.SemaphoreType.DMA((8,)),
            pltpu.SemaphoreType.DMA((n_tok // _LANES,)),
        ],
        compiler_params=pltpu.CompilerParams(vmem_limit_bytes=110 * 1024 * 1024),
    )(A_x.reshape(n_tok, d_model).T, A_mem0.reshape(n_mem, d_model), A_Wq, A_Wk, A_Wv,
      A_Wo.transpose(0, 2, 1), B_w1, B_w3, B_w2.T)
    return out_t.T.reshape(A_x.shape)
```
